```python
import os as _os
_os.environ.setdefault("JAX_PLATFORMS", "cpu")
import jax
import jax.numpy as jnp

def _softmax(x, axis=-1):
    return jax.nn.softmax(x, axis=axis)
def _gelu(x):
    return jax.nn.gelu(x, approximate=True)
def _silu(x):
    return jax.nn.silu(x)
def _sigmoid(x):
    return jax.nn.sigmoid(x)
def _layernorm(x, axis=-1, eps=1e-5):
    m = jnp.mean(x, axis=axis, keepdims=True)
    v = jnp.var(x, axis=axis, keepdims=True)
    return (x - m) / jnp.sqrt(v + eps)
def _scatter_add(tgt, idx, src, axis=0):
    return tgt.at[idx].add(src)
def _segment_sum(src, seg, n):
    return jax.ops.segment_sum(src, seg, n)
class _Rng:
    def __init__(self, key):
        self._k = key
    def _next(self):
        self._k, sub = jax.random.split(self._k)
        return sub
    def normal(self, shape):
        return jax.random.normal(self._next(), shape, dtype=jnp.bfloat16)
    def randint(self, lo, hi, shape):
        return jax.random.randint(self._next(), shape, lo, hi, dtype=jnp.int32)
    def uniform(self, shape, lo=0.0, hi=1.0):
        return jax.random.uniform(self._next(), shape, jnp.bfloat16, lo, hi)
    def permutation(self, n):
        return jax.random.permutation(self._next(), n)


kernel_name = 'concat_heads__mha_block__ssm_conv_s4__prompt'

def setup_inputs():
    _rng = _Rng(jax.random.key(int.from_bytes(__import__("os").urandom(4), "little")))
    _w = (lambda a: (lambda t: t.astype(jnp.bfloat16) if jnp.issubdtype(t.dtype, jnp.floating) else t)(jnp.asarray(a)))
    def _A_setup():
        B, S, D, H = 1, 2048, 448, 16
        return {
            "x": _w((lambda *s: _rng.normal(s) * 0.2)(B, S, D)),
            "wqkv": _w((lambda *s: _rng.normal(s) * 0.2)(D, 3 * D)),
            "wo": _w((lambda *s: _rng.normal(s) * 0.05)(D, D)),
        }
    _A_in = _A_setup()

    def _B_setup():
        B, L, D, N = 1, 2048, 448, 256
        A_re = -jnp.exp((lambda *s: _rng.normal(s) * 0.2)(D, N))
        A_im = jnp.pi * (lambda *s: _rng.normal(s) * 0.2)(D, N)
        B_re = (lambda *s: _rng.normal(s) * 0.2)(D, N)
        B_im = (lambda *s: _rng.normal(s) * 0.2)(D, N)
        C_re = (lambda *s: _rng.normal(s) * 0.2)(D, N)
        C_im = (lambda *s: _rng.normal(s) * 0.2)(D, N)
        log_dt = (lambda *s: _rng.normal(s) * 0.2)(D) * 0.5 - 4.0
        Dskip = (lambda *s: _rng.normal(s) * 0.05)(D)
        return {
            "u": _w((lambda *s: _rng.normal(s) * 0.05)(B, L, D)),
            "A_re": _w(A_re),
            "A_im": _w(A_im),
            "B_re": _w(B_re),
            "B_im": _w(B_im),
            "C_re": _w(C_re),
            "C_im": _w(C_im),
            "log_dt": _w(log_dt),
            "Dskip": _w(Dskip),
        }
    _B_in = _B_setup()

    return {
        "A_x": _A_in["x"],
        "A_wqkv": _A_in["wqkv"],
        "A_wo": _A_in["wo"],
        "B_u": _B_in["u"],
        "B_A_re": _B_in["A_re"],
        "B_A_im": _B_in["A_im"],
        "B_B_re": _B_in["B_re"],
        "B_B_im": _B_in["B_im"],
        "B_C_re": _B_in["C_re"],
        "B_C_im": _B_in["C_im"],
        "B_log_dt": _B_in["log_dt"],
        "B_Dskip": _B_in["Dskip"],
    }

def reference(A_x, A_wqkv, A_wo, B_u, B_A_re, B_A_im, B_B_re, B_B_im, B_C_re, B_C_im, B_log_dt, B_Dskip):
    def _A_ref(x, wqkv, wo):
        B, S, D = x.shape
        H = 16
        Dh = D // H
        qkv = (lambda x, *d: x.transpose(*d))((x @ wqkv).reshape(B, S, 3, H, Dh), 2, 0, 3, 1, 4)
        q, k, v = qkv[0], qkv[1], qkv[2]
        scores = jnp.einsum("bhqd,bhkd->bhqk", q, k) * (Dh ** -0.5)
        p = _softmax(scores, axis=-1)
        o = jnp.einsum("bhqk,bhkd->bhqd", p, v)
        return (lambda x, *d: x.transpose(*d))(o, 0, 2, 1, 3).reshape(B, S, D) @ wo

    def _B_ref(u, A_re, A_im, B_re, B_im, C_re, C_im, log_dt, Dskip):
        Bsz, L, D = u.shape
        dt = jnp.exp(log_dt)[:, None]
        A = A_re + 1j * A_im
        Bc = B_re + 1j * B_im
        Cc = C_re + 1j * C_im
        logdA = dt * A
        dB = dt * Bc
        l = (lambda x, dt: x.astype(dt))(jnp.arange(L), A_re.dtype)
        P = jnp.exp(logdA[:, :, None] * l[None, None, :])
        K = jnp.einsum("dn,dnl,dn->dl", Cc, P, dB).real
        L2 = 2 * L
        Kp = jnp.pad(K, ((0, 0), (0, L)))
        up = (lambda x, *d: x.transpose(*d))(u, 0, 2, 1)
        up = jnp.pad(up, ((0, 0), (0, 0), (0, L)))
        Kf = (lambda x, axes=(-2,-1): jnp.fft.rfft2(x.astype(jnp.float32), axes=axes))(Kp[:, None, :], axes=(-2, -1))
        Uf = (lambda x, axes=(-2,-1): jnp.fft.rfft2(x.astype(jnp.float32), axes=axes))(up[:, :, None, :], axes=(-2, -1))
        Yf = Uf * Kf[None, :, :, :]
        y = (lambda x, s, axes=(-2,-1): jnp.fft.irfft2(x, s=s, axes=axes).astype(jnp.bfloat16))(Yf, (1, L2), axes=(-2, -1))[:, :, 0, :L]
        y = (lambda x, *d: x.transpose(*d))(y, 0, 2, 1) + u * Dskip[None, None, :]
        return y

    a = _A_ref(A_x, A_wqkv, A_wo)
    b = _B_ref(B_u, B_A_re, B_A_im, B_B_re, B_B_im, B_C_re, B_C_im, B_log_dt, B_Dskip)
    return jnp.concatenate([a, b], axis=-1)
```

```python
import functools
import numpy as np
import ml_dtypes
import jax
import jax.numpy as jnp
from jax import lax
from jax.experimental import pallas as pl
from jax.experimental.pallas import tpu as pltpu

bf = jnp.bfloat16
f32 = jnp.float32

SEQ = 2048
D = 448
H = 16
DH = 28
NST = 256
BQ = 512
CK = 128
NQB = SEQ // BQ
LOG2E = 1.4426950408889634

_L1 = np.array([0, 1, 2, 3, 4, 5, 6, 7, 512, 516, 1024, 1536, 2048])


def _slabs(j):
    if j < 2:
        return [(r, 16 * j) for r in range(8)]
    if j < 4:
        return [(r, 16 * j) for r in (0, 2, 4, 6)] + [(0, 48) if j == 2 else (8, 0)]
    if j < 8:
        return [(8, 16 * (j - 4)), (9, 16 * (j - 4))] + [(8, 16 * (j - 3)) if j < 7 else (10, 0)]
    if j < 12:
        return [(10, 16 * (j - 8))] + [(10, 16 * (j - 7)) if j < 11 else (11, 0)]
    return [(11, 16 * (j - 12))] + [(11, 16 * (j - 11)) if j < 15 else (12, 0)]


def _group(j):
    return 0 if j < 2 else 1 if j < 4 else 2 if j < 8 else 3


def _make_consts():
    k = np.arange(128)[:, None]
    n = np.arange(128)[None, :]
    ang = np.pi * (2 * k + 1) * n / 256.0
    ct = np.concatenate([np.cos(ang), -np.sin(ang)], 0)
    n2 = (128 + np.arange(128))[:, None]
    k2 = np.arange(128)[None, :]
    ang2 = np.pi * (2 * k2 + 1) * n2 / 256.0
    ci = np.concatenate([np.cos(ang2), -np.sin(ang2)], 1) / 128.0
    n2 = np.arange(128)[:, None]
    ang2 = np.pi * (2 * k2 + 1) * n2 / 256.0
    ci = np.concatenate([np.cos(ang2), -np.sin(ang2)], 1) / 128.0
    out = np.zeros((6, 256, 128), np.float64)
    out[0] = ct
    for g, j in enumerate((0, 2, 4, 8)):
        pos = {}
        sl = _slabs(j)
        for si, (rho, c0) in enumerate(sl):
            for cc in range(16):
                pos.setdefault(int(_L1[rho] + 8 * (c0 + cc)), si * 16 + cc)
        m = np.zeros((256, 128))
        for nn in range(128):
            lr = int(np.float32(128 * j + nn).astype(ml_dtypes.bfloat16).astype(np.float32))
            m[:, pos[lr]] += ct[:, nn]
        out[g + 1] = m
    out[5, 0:128] = ci[:, 0:128]
    out[5, 128:256] = ci[:, 128:256]
    return out.astype(np.float32).astype(ml_dtypes.bfloat16)


_CONSTS = _make_consts()
_WIN = (128, 80, 48, 32)


def _cmul(ar, ai, br, bi):
    return ar * br - ai * bi, ar * bi + ai * br


def _cmulc(ar, ai, br, bi):
    return ar * br + ai * bi, ai * br - ar * bi


def _csq(ar, ai):
    return ar * ar - ai * ai, (ar + ar) * ai


_FLAGS = None
_OPT = OPQ
XP = 516
NPIN_C = _OPT.get("npin_c", 4)
NPIN_G = _OPT.get("npin_g", 1)


def _slab_rows(j):
    sl = _slabs(j)
    rows = [64 * rho + c0 for rho, c0 in sl]
    return rows + [rows[0]] * (8 - len(rows))


def _kernel(xT_h, wqkv_h, wo_h, uT_h, are_h, aim_h, bre_h, bim_h, cre_h, cim_h, ldt_h, dsk_h, cst_h,
            out_h,
            xT_v, wqkv_v, wo_v, uT_s, par_v, ldt_v, dsk_v, cst_v,
            wt0, wt1, wt2, wt3, wp_s, wo_f, wop_s,
            q_s, k_s, v_s, s_s, o_s,
            pw, gs0, gs1, xk_s, kct_s,
            kuh, yf_s, st_s, tab_s, sems, osem):
    cp_w = pltpu.make_async_copy(wqkv_h, wqkv_v, sems.at[0])
    cp_x = [pltpu.make_async_copy(xT_h.at[:, pl.ds(512 * b, 512)], xT_v.at[:, pl.ds(512 * b, 512)], sems.at[13 + b])
            for b in range(4)]
    cp_par = [pltpu.make_async_copy(r, par_v.at[i], sems.at[2 + i])
              for i, r in enumerate((are_h, aim_h, bre_h, bim_h, cre_h, cim_h))]
    cp_ldt = pltpu.make_async_copy(ldt_h, ldt_v, sems.at[8])
    cp_dsk = pltpu.make_async_copy(dsk_h, dsk_v, sems.at[9])
    cp_cst = pltpu.make_async_copy(cst_h, cst_v, sems.at[10])
    cp_wo = pltpu.make_async_copy(wo_h, wo_v, sems.at[11])
    cp_u = pltpu.make_async_copy(uT_h, uT_s.at[pl.ds(64, D), :], sems.at[12])
    cp_w.start()
    cp_x[0].start()
    cp_x[1].start()
    for c in cp_par:
        c.start()
    cp_ldt.start()
    cp_x[2].start()
    cp_x[3].start()
    cp_dsk.start()
    cp_cst.start()
    cp_wo.start()
    cp_u.start()

    nt = (((1,), (1,)), ((), ()))
    tn = (((0,), (0,)), ((), ()))
    PR, PI, ER, EI, MU, ONE = 0, 96, 192, 384, 576, 624

    uT_s[0:64, :] = jnp.zeros((64, SEQ), bf)
    for j in range(16):
        for si, r in enumerate(_slab_rows(j)):
            tab_s[j * 8 + si] = np.int32(r)
    gss = (gs0, gs1)
    for st in range(2):
        for t in range(2):
            gss[st][t, ER + 13 * 12:ER + 16 * 12, :] = jnp.zeros((36, 128), f32)
            gss[st][t, EI + 13 * 12:EI + 16 * 12, :] = jnp.zeros((36, 128), f32)
            gss[st][t, ONE:ONE + 16, :] = jnp.ones((16, 128), f32)
    for rho in range(16):
        xk_s[XP * rho:XP * rho + 64, :] = jnp.zeros((64, 64), f32)
    yf_s[0] = jnp.zeros((4, 256, 128), f32)

    cp_w.wait()
    wT = wqkv_v[...].T.astype(f32)
    wts = (wt0, wt1, wt2, wt3)
    for t in range(4):
        w = 64 if t == 3 else 128
        wts[t][0:1344, :] = wT[:, 128 * t:128 * t + w]
        wts[t][1344:1352, :] = jnp.zeros((8, w), f32)
    r32 = lax.broadcasted_iota(jnp.int32, (32, D), 0)
    for hh in range(48):
        slab = jnp.concatenate([wts[t][pl.ds(28 * hh, 32), :] for t in range(4)], axis=1)
        if hh < 16:
            slab = jnp.where(r32 < DH, slab, np.float32(0.0))
        wp_s[32 * hh:32 * hh + 32, :] = slab.astype(bf)

    def bprep(r0, n, dt_col):
        sl = slice(r0, r0 + n)
        dt2 = jnp.concatenate([dt_col[sl], dt_col[sl]], axis=1)
        zr = dt2 * par_v[0, sl, :].astype(f32)
        zi = dt2 * par_v[1, sl, :].astype(f32)
        dbr = dt2 * par_v[2, sl, :].astype(f32)
        dbi = dt2 * par_v[3, sl, :].astype(f32)
        cr = par_v[4, sl, :].astype(f32)
        ci_ = par_v[5, sl, :].astype(f32)
        wr_, wi_ = _cmul(cr, ci_, dbr, dbi)
        pw[2, sl, :] = wr_
        pw[3, sl, :] = wi_
        mag = jnp.exp(zr)
        pw[0, sl, :] = mag * jnp.cos(zi)
        pw[1, sl, :] = mag * jnp.sin(zi)

    rowv = lax.broadcasted_iota(jnp.int32, (512, 512), 0)
    dt_col = None
    for b in range(4):
        cp_x[b].wait()
        if b == 1:
            for c in cp_par:
                c.wait()
            cp_ldt.wait()
            ldt = ldt_v[...].astype(f32).reshape(1, D)
            dt_row = jnp.exp(ldt).astype(bf).astype(f32)
            dt_col = jnp.broadcast_to(dt_row, (128, D)).T
        ts = slice(512 * b, 512 * b + 512)
        xb = xT_v[:, ts]
        kT = jnp.dot(wp_s[512:1024, :], xb, preferred_element_type=f32).astype(bf)
        qq = jnp.dot(wp_s[0:512, :], xb, preferred_element_type=f32)
        qq = (qq * np.float32(DH ** -0.5 * LOG2E)).astype(bf)
        for hh in range(16):
            q_s[hh, :, ts] = qq[32 * hh:32 * hh + 32, :]
        vv = jnp.dot(wp_s[1024:1536, :], xb, preferred_element_type=f32)
        vv = jnp.where((rowv % 32) == 28, np.float32(1.0), vv).astype(bf)
        for hh in range(16):
            v_s[hh, :, ts] = vv[32 * hh:32 * hh + 32, :]
        for g in range(4):
            kg = kT[128 * g:128 * g + 128, :].T
            k_s[4 * g, ts, :] = kg
            for j in range(1, 4):
                k_s[4 * g + j, ts, :] = pltpu.roll(kg, 128 - 32 * j, 1)
        if b >= 1:
            r0 = (0, 0, 152, 304)[b]
            n = (0, 152, 152, 144)[b]
            bprep(r0, n, dt_col)

    cp_cst.wait()
    cp_u.wait()
    cp_dsk.wait()
    cp_wo.wait()
    wo_f[...] = wo_v[...].astype(f32)
    for hh in range(16):
        wop_s[32 * hh:32 * hh + 32, :] = jnp.concatenate(
            [wo_f[28 * hh:28 * hh + 28, :], jnp.zeros((4, D), f32)], axis=0).astype(bf)

    def kgen_prep(b, st):
        d0 = pl.multiple_of(b * 8, 8)
        gs = gss[st]

        def ld_e1():
            return pw[0, pl.ds(d0, 8), :], pw[1, pl.ds(d0, 8), :]

        def ld_w():
            return pw[2, pl.ds(d0, 8), :], pw[3, pl.ds(d0, 8), :]

        def tmp_ld(k):
            return pw[4, 48 * st + 16 * k:48 * st + 16 * k + 8, :], pw[4, 48 * st + 16 * k + 8:48 * st + 16 * k + 16, :]

        def tmp_st(k, v):
            pw[4, 48 * st + 16 * k:48 * st + 16 * k + 8, :] = v[0]
            pw[4, 48 * st + 16 * k + 8:48 * st + 16 * k + 16, :] = v[1]

        def put(base_r, base_i, idx, val):
            for t in range(2):
                sl = slice(128 * t, 128 * t + 128)
                gs[t, base_r + 12 * idx:base_r + 12 * idx + 8, :] = val[0][:, sl]
                gs[t, base_i + 12 * idx:base_i + 12 * idx + 8, :] = val[1][:, sl]

        def get(base_r, base_i, idx):
            return (jnp.concatenate([gs[t, base_r + 12 * idx:base_r + 12 * idx + 8, :] for t in range(2)], axis=1),
                    jnp.concatenate([gs[t, base_i + 12 * idx:base_i + 12 * idx + 8, :] for t in range(2)], axis=1))

        def putm(mi, val):
            for t in range(2):
                sl = slice(128 * t, 128 * t + 128)
                gs[t, MU + 16 * mi:MU + 16 * mi + 8, :] = val[0][:, sl]
                gs[t, MU + 16 * mi + 8:MU + 16 * mi + 16, :] = val[1][:, sl]

        def getm(mi):
            return (jnp.concatenate([gs[t, MU + 16 * mi:MU + 16 * mi + 8, :] for t in range(2)], axis=1),
                    jnp.concatenate([gs[t, MU + 16 * mi + 8:MU + 16 * mi + 16, :] for t in range(2)], axis=1))
        e1, w = ld_e1(), ld_w()
        put(ER, EI, 0, w)
        put(ER, EI, 1, _cmul(*w, *e1))
        e2 = _csq(*e1)
        put(ER, EI, 2, _cmul(*w, *e2))
        tmp_st(0, e2)
        e3 = _cmul(*e2, *e1)
        tmp_st(1, e3)
        yield
        w, e2, e3 = ld_w(), tmp_ld(0), tmp_ld(1)
        put(ER, EI, 3, _cmul(*w, *e3))
        e4 = _csq(*e2)
        tmp_st(2, e4)
        put(ER, EI, 4, _cmul(*w, *e4))
        e6 = _csq(*e3)
        put(ER, EI, 6, _cmul(*w, *e6))
        yield
        e1, w, e3, e4 = ld_e1(), ld_w(), tmp_ld(1), tmp_ld(2)
        put(ER, EI, 5, _cmul(*w, *_cmul(*e4, *e1)))
        put(ER, EI, 7, _cmul(*w, *_cmul(*e4, *e3)))
        e8 = _csq(*e4)
        put(PR, PI, 0, (jnp.ones_like(e8[0]), jnp.zeros_like(e8[0])))
        put(PR, PI, 1, (e8[0], -e8[1]))
        yield
        p1 = get(PR, PI, 1)
        p2 = _csq(*p1)
        put(PR, PI, 2, p2)
        p3 = _cmul(*p2, *p1)
        put(PR, PI, 3, p3)
        p4 = _csq(*p2)
        put(PR, PI, 4, p4)
        put(PR, PI, 5, _cmul(*p4, *p1))
        put(PR, PI, 6, _csq(*p3))
        yield
        p3, p4 = get(PR, PI, 3), get(PR, PI, 4)
        put(PR, PI, 7, _cmul(*p4, *p3))
        m8 = _csq(*p4)
        putm(0, m8)
        m16 = _csq(*m8)
        putm(1, m16)
        m32 = _csq(*m16)
        putm(2, m32)
        yield
        w, e4, m32 = ld_w(), tmp_ld(2), getm(2)
        x512c = _csq(*m32)
        w512 = _cmulc(*w, *x512c)
        put(ER, EI, 8, w512)
        put(ER, EI, 9, _cmul(*w512, *e4))
        x1024c = _csq(*x512c)
        put(ER, EI, 10, _cmulc(*w, *x1024c))
        put(ER, EI, 11, _cmulc(*w, *_cmul(*x1024c, *x512c)))
        put(ER, EI, 12, _cmulc(*w, *_csq(*x1024c)))
        yield

    def kgen_chan(b, i, st):
        d0 = b * 8
        gs = gss[st]
        e2t_r, e2t_i, e1_r, e1_i = [], [], [], []
        for t in range(2):
            b0 = (gs[t, pl.ds(PR + i, 8, stride=12), :], gs[t, pl.ds(PI + i, 8, stride=12), :])

            def mul(mi):
                return (jnp.broadcast_to(gs[t, pl.ds(MU + 16 * mi + i, 1), :], (8, 128)),
                        jnp.broadcast_to(gs[t, pl.ds(MU + 16 * mi + 8 + i, 1), :], (8, 128)))
            mm8, mm16, mm32 = mul(0), mul(1), mul(2)
            b1 = _cmul(*b0, *mm8)
            b2 = _cmul(*b0, *mm16)
            b3 = _cmul(*b1, *mm16)
            b4 = _cmul(*b0, *mm32)
            b5 = _cmul(*b1, *mm32)
            b6 = _cmul(*b2, *mm32)
            b7 = _cmul(*b3, *mm32)
            blks = (b0, b1, b2, b3, b4, b5, b6, b7)
            e2t_r.append(jnp.concatenate([bb[0] for bb in blks], axis=0))
            e2t_i.append(jnp.concatenate([bb[1] for bb in blks], axis=0))
            e1_r.append(gs[t, pl.ds(ER + i, 16, stride=12), :])
            e1_i.append(gs[t, pl.ds(EI + i, 16, stride=12), :])
            if t == 0:
                yield
        lhs = jnp.concatenate(e1_r + e1_i, axis=1).astype(bf)
        rhs = jnp.concatenate(e2t_r + e2t_i, axis=1).astype(bf)
        kc = lax.dot_general(lhs, rhs, nt, preferred_element_type=f32)
        xk_s[pl.ds(64 + d0 + i, 16, stride=XP), :] = kc
        yield

    def u_fwd(a):
        t0 = pl.multiple_of(a * 128, 128)
        aa = lax.dot_general(cst_v[0], uT_s[:, pl.ds(t0, 128)], nt, preferred_element_type=f32)
        for lt in range(4):
            kuh[1, lt, a] = aa[:, 128 * lt:128 * lt + 128]

    def k_tr(rho):
        r0 = pl.multiple_of(rho * XP, 4)
        c0 = pl.multiple_of(rho * 64, 64)
        kct_s[pl.ds(c0, 64), :] = xk_s[pl.ds(r0, 512), :].astype(bf).T

    def k_fwd(j):
        g = jnp.where(j < 2, 1, jnp.where(j < 4, 2, jnp.where(j < 8, 3, 4)))
        win = jnp.concatenate(
            [kct_s[pl.ds(pl.multiple_of(tab_s[j * 8 + si], 16), 16), :] for si in range(8)], axis=0)
        kk = jnp.dot(cst_v[g], win, preferred_element_type=f32)
        for lt in range(4):
            kuh[0, lt, j] = kk[:, 128 * lt:128 * lt + 128]

    def conv_pair(unit, p, nsplit):
        lt = unit // 16
        r0 = pl.multiple_of((unit % 16) * 8, 8)
        a0 = 2 * p
        a1 = 2 * p + 1
        ar0 = ai0 = ar1 = ai1 = None
        uprev = None
        cuts = set(int(round((a1 + 1) * k / nsplit)) for k in range(1, nsplit))
        for j in range(a1 + 1):
            if j in cuts:
                yield
            kr = kuh[0, lt, j, pl.ds(r0, 8), :]
            ki = kuh[0, lt, j, pl.ds(128 + r0, 8), :]
            m1 = a1 - j
            if uprev is None:
                u1 = (kuh[1, lt, m1, pl.ds(r0, 8), :], kuh[1, lt, m1, pl.ds(128 + r0, 8), :])
            else:
                u1 = uprev
            tr = kr * u1[0] - ki * u1[1]
            ti = kr * u1[1] + ki * u1[0]
            ar1 = tr if ar1 is None else ar1 + tr
            ai1 = ti if ai1 is None else ai1 + ti
            m0 = a0 - j
            if m0 >= 0:
                u0 = (kuh[1, lt, m0, pl.ds(r0, 8), :], kuh[1, lt, m0, pl.ds(128 + r0, 8), :])
                tr = kr * u0[0] - ki * u0[1]
                ti = kr * u0[1] + ki * u0[0]
                ar0 = tr if ar0 is None else ar0 + tr
                ai0 = ti if ai0 is None else ai0 + ti
                uprev = u0
        for a, (yr, yi) in ((a0, (ar0, ai0)), (a1, (ar1, ai1))):
            yf_s[a + 1, lt, pl.ds(r0, 8), :] = yr
            yf_s[a + 1, lt, pl.ds(128 + r0, 8), :] = yi
        yield

    cim = jnp.concatenate([cst_v[5, 0:128, :], cst_v[5, 128:256, :]], axis=1)
    sgn = jnp.where(lax.broadcasted_iota(jnp.int32, (128, 128), 0) % 2 == 0, np.float32(1.0), np.float32(-1.0))

    def inverse(a):
        t0 = pl.multiple_of(a * 128, 128)
        parts = []
        for lt in range(4):
            yr = yf_s[a + 1, lt, 0:128, :] - sgn * yf_s[a, lt, 128:256, :]
            yi = yf_s[a + 1, lt, 128:256, :] + sgn * yf_s[a, lt, 0:128, :]
            parts.append(jnp.concatenate([yr, yi], axis=0).astype(bf))
        yy = jnp.concatenate(parts, axis=1)
        y = jnp.dot(cim, yy, preferred_element_type=f32).astype(bf)
        st_s[pl.ds(t0, 128), 448:512] = y[:, 64:128]
        st_s[pl.ds(t0, 128), 512:896] = y[:, 128:512]

    NB = NQB * H
    NC = SEQ // CK

    def q_of(i):
        qb = i // H
        h = i % H
        q0 = pl.multiple_of(qb * BQ, BQ)
        return q_s[h, :, pl.ds(q0, BQ)], h

    def pv_chunk(h, c, m, acc):
        s = s_s[pl.ds(c * CK, CK), :]
        p = jnp.exp2(s - m).astype(bf)
        o = jnp.dot(v_s[h, :, pl.ds(c * CK, CK)], p, preferred_element_type=f32)
        return o if acc is None else acc + o

    def qk_chunk(h, qm, c, mrun, pins=None, tasks=()):
        s = jnp.dot(k_s[h, pl.ds(c * CK, CK), 0:32], qm, preferred_element_type=f32)
        s_s[pl.ds(c * CK, CK), :] = s
        mm = jnp.max(s.reshape(CK // 8, 8, BQ), axis=0)
        if pins is not None:
            pin_store, npin, pinned = pins
            for k in range(npin):
                g = (k + 1) * (CK // 8) // npin - 1 if npin > 1 else _OPT.get("pin1_g", 3)
                pin_store(s[8 * g:8 * g + 8, 0:128])
                for t in pinned:
                    next(t, None)
            for t in pinned:
                for _ in t:
                    pass
        for t in tasks:
            for _ in t:
                pass
        return mm if mrun is None else jnp.maximum(mrun, mm)

    qm0, h0 = q_of(0)
    mrun = None
    for c in range(NC):
        mrun = qk_chunk(0, qm0, c, mrun)
    for _ in kgen_prep(0, 0):
        pass

    def make_step(extra):
        def att_step(i, mrun_prev):
            m_cur = jnp.max(mrun_prev, axis=0, keepdims=True)
            inext = jnp.minimum(i + 1, NB - 1)
            qm, hn = q_of(inext)
            qb = i // H
            h = i % H
            mrun = None
            acc = None
            state = {}
            for c in range(NC):
                acc = pv_chunk(h, c, m_cur, acc)
                pins, tasks = (None, ()) if extra is None else extra(i, c, state)
                mrun = qk_chunk(hn, qm, c, mrun, pins, tasks)
            inv = 1.0 / acc[28:29, :]
            q0 = pl.multiple_of(qb * BQ, BQ)
            o_s[h, :, pl.ds(q0, BQ)] = (acc * inv).astype(bf)
            return mrun
        return att_step

    def opaque(i, k):
        return (i * k) >> 12

    def fn_task(fn, *a):
        def g():
            fn(*a)
            yield
        return g()

    def ex_G(i, c, state, with_u=False):
        st = c // 8
        dz = pl.multiple_of(448 + opaque(i, 9) * 8, 8)

        def pin_store(v):
            pw[4, pl.ds(dz, 8), 0:128] = v
        tasks = [kgen_chan(2 * i + st, c % 8, st)]
        pinned = []
        if c % 8 == 0:
            nb = 2 * i + 1 if st == 0 else jnp.minimum(2 * i + 2, D // 8 - 1)
            state['prep'] = kgen_prep(nb, 1 - st)
        if c % 8 < 6:
            pinned.append(fn_task(next, state['prep']))
        if with_u and c == 4:
            tasks.append(fn_task(u_fwd, i))
        if NPIN_G == 0 or not pinned:
            return None, pinned + tasks
        return (pin_store, NPIN_G, pinned), tasks

    def ex_GU(i, c, state):
        return ex_G(i, c, state, True)

    def ex_T(i, c, state):
        if c % 4 == 1:
            return None, [fn_task(k_tr, (i - 28) * 4 + c // 4)]
        return None, []

    def ex_KF(i, c, state):
        if c % 4 == 1:
            return None, [fn_task(k_fwd, (i - 32) * 4 + c // 4)]
        return None, []

    def ex_C(i, c, state):
        dz = 16 + opaque(i, 9)

        def pin_store(v):
            kuh[0, 0, dz, 0:8, :] = v
        ub = (i - 36) * 4 + c // 4
        pp = c % 4
        return (pin_store, NPIN_C, [conv_pair(ub, pp, NPIN_C), conv_pair(ub, 7 - pp, NPIN_C)]), []

    def ex_I(i, c, state):
        if c % 8 == 2:
            return None, [fn_task(inverse, (i - 52) * 2 + c // 8)]
        return None, []

    out_cps = []

    def outproj(qb):
        oT = o_s[:, :, qb * BQ:(qb + 1) * BQ].reshape(512, BQ)
        ya = lax.dot_general(oT, wop_s[...], tn, preferred_element_type=f32)
        st_s[qb * BQ:(qb + 1) * BQ, 0:448] = ya.astype(bf)

    def out_dma(r0, n, k):
        cp = pltpu.make_async_copy(st_s.at[pl.ds(r0, n), :], out_h.at[0, pl.ds(r0, n), :], osem.at[k])
        cp.start()
        out_cps.append(cp)

    mrun = lax.fori_loop(0, 16, make_step(ex_GU), mrun)
    outproj(0)
    mrun = lax.fori_loop(16, 28, make_step(ex_G), mrun)
    mrun = lax.fori_loop(28, 32, make_step(ex_T), mrun)
    outproj(1)
    mrun = lax.fori_loop(32, 36, make_step(ex_KF), mrun)
    dsk = jnp.concatenate([jnp.zeros((1, 64), f32), dsk_v[...].astype(f32).reshape(1, D)], axis=1)
    for lt in range(4):
        kuh[0, lt, 0, 0:128, :] = kuh[0, lt, 0, 0:128, :] + dsk[:, 128 * lt:128 * lt + 128]
    mrun = lax.fori_loop(36, 48, make_step(ex_C), mrun)
    outproj(2)
    mrun = lax.fori_loop(48, 52, make_step(ex_C), mrun)
    mrun = lax.fori_loop(52, 60, make_step(ex_I), mrun)
    out_dma(0, 3 * BQ, 0)
    mrun = lax.fori_loop(60, 64, make_step(None), mrun)
    outproj(3)
    out_dma(3 * BQ, BQ, 1)
    for cp in out_cps:
        cp.wait()


@jax.jit
def pallas_concat_heads__mha_block__ssm_conv_s4__prompt_kernel(
        A_x, A_wqkv, A_wo, B_u, B_A_re, B_A_im, B_B_re, B_B_im, B_C_re, B_C_im, B_log_dt, B_Dskip):
    hbm = pl.BlockSpec(memory_space=pltpu.HBM)
    scratch = [
        pltpu.VMEM((D, SEQ), bf),
        pltpu.VMEM((D, 3 * D), bf),
        pltpu.VMEM((D, D), bf),
        pltpu.VMEM((512, SEQ), bf),
        pltpu.VMEM((6, D, NST), bf),
        pltpu.VMEM((D,), bf),
        pltpu.VMEM((D,), bf),
        pltpu.VMEM((6, 256, 128), bf),
        pltpu.VMEM((1352, 128), f32), pltpu.VMEM((1352, 128), f32),
        pltpu.VMEM((1352, 128), f32), pltpu.VMEM((1352, 64), f32),
        pltpu.VMEM((1536, D), bf),
        pltpu.VMEM((D, D), f32),
        pltpu.VMEM((512, D), bf),
        pltpu.VMEM((16, 32, SEQ), bf),
        pltpu.VMEM((16, SEQ, 128), bf),
        pltpu.VMEM((16, 32, SEQ), bf),
        pltpu.VMEM((SEQ, BQ), f32),
        pltpu.VMEM((16, 32, SEQ), bf),
        pltpu.VMEM((5, 456, NST), f32),
        pltpu.VMEM((2, 640, 128), f32), pltpu.VMEM((2, 640, 128), f32),
        pltpu.VMEM((XP * 16, 64), f32),
        pltpu.VMEM((1024, 512), bf),
        pltpu.VMEM((2, 4, 17, 256, 128), f32),
        pltpu.VMEM((17, 4, 256, 128), f32),
        pltpu.VMEM((SEQ, 896), bf),
        pltpu.SMEM((128,), jnp.int32),
        pltpu.SemaphoreType.DMA((17,)),
        pltpu.SemaphoreType.DMA((2,)),
    ]
    c = lambda a: pltpu.with_memory_space_constraint(a, pltpu.HBM)
    xT = jnp.transpose(A_x[0])
    uT = jnp.transpose(B_u[0])
    args = [c(a) for a in (xT, A_wqkv, A_wo, uT, B_A_re, B_A_im, B_B_re, B_B_im, B_C_re, B_C_im,
                           B_log_dt, B_Dskip, jnp.asarray(_CONSTS))]
    return pl.pallas_call(
        _kernel,
        out_shape=jax.ShapeDtypeStruct((1, SEQ, 2 * D), bf),
        in_specs=[hbm] * 13,
        out_specs=hbm,
        scratch_shapes=scratch,
        compiler_params=pltpu.CompilerParams(vmem_limit_bytes=110 * 2 ** 20, flags=_FLAGS),
    )(*args)
```

```python
import functools
import numpy as np
import ml_dtypes
import jax
import jax.numpy as jnp
from jax import lax
from jax.experimental import pallas as pl
from jax.experimental.pallas import tpu as pltpu

bf = jnp.bfloat16
f32 = jnp.float32

SEQ = 2048
D = 448
H = 16
DH = 28
NST = 256
BQ = 512
CK = 128
NQB = SEQ // BQ
LOG2E = 1.4426950408889634

_L1 = np.array([0, 1, 2, 3, 4, 5, 6, 7, 512, 516, 1024, 1536, 2048])


def _slabs(j):
    if j < 2:
        return [(r, 16 * j) for r in range(8)]
    if j < 4:
        return [(r, 16 * j) for r in (0, 2, 4, 6)] + [(0, 48) if j == 2 else (8, 0)]
    if j < 8:
        return [(8, 16 * (j - 4)), (9, 16 * (j - 4))] + [(8, 16 * (j - 3)) if j < 7 else (10, 0)]
    if j < 12:
        return [(10, 16 * (j - 8))] + [(10, 16 * (j - 7)) if j < 11 else (11, 0)]
    return [(11, 16 * (j - 12))] + [(11, 16 * (j - 11)) if j < 15 else (12, 0)]


def _group(j):
    return 0 if j < 2 else 1 if j < 4 else 2 if j < 8 else 3


def _make_consts():
    k = np.arange(128)[:, None]
    n = np.arange(128)[None, :]
    ang = np.pi * (2 * k + 1) * n / 256.0
    ct = np.concatenate([np.cos(ang), -np.sin(ang)], 0)
    n2 = (128 + np.arange(128))[:, None]
    k2 = np.arange(128)[None, :]
    ang2 = np.pi * (2 * k2 + 1) * n2 / 256.0
    ci = np.concatenate([np.cos(ang2), -np.sin(ang2)], 1) / 128.0
    n2 = np.arange(128)[:, None]
    ang2 = np.pi * (2 * k2 + 1) * n2 / 256.0
    ci = np.concatenate([np.cos(ang2), -np.sin(ang2)], 1) / 128.0
    out = np.zeros((6, 256, 128), np.float64)
    out[0] = ct
    for g, j in enumerate((0, 2, 4, 8)):
        pos = {}
        sl = _slabs(j)
        for si, (rho, c0) in enumerate(sl):
            for cc in range(16):
                pos.setdefault(int(_L1[rho] + 8 * (c0 + cc)), si * 16 + cc)
        m = np.zeros((256, 128))
        for nn in range(128):
            lr = int(np.float32(128 * j + nn).astype(ml_dtypes.bfloat16).astype(np.float32))
            m[:, pos[lr]] += ct[:, nn]
        out[g + 1] = m
    out[5, 0:128] = ci[:, 0:128]
    out[5, 128:256] = ci[:, 128:256]
    return out.astype(np.float32).astype(ml_dtypes.bfloat16)


_CONSTS = _make_consts()
_WIN = (128, 80, 48, 32)


def _cmul(ar, ai, br, bi):
    return ar * br - ai * bi, ar * bi + ai * br


def _cmulc(ar, ai, br, bi):
    return ar * br + ai * bi, ai * br - ar * bi


def _csq(ar, ai):
    return ar * ar - ai * ai, (ar + ar) * ai


_FLAGS = None
_OPT = OPQ
import contextlib as _ctx
_SC = _OPT.get('scopes', False)
def _scope(n):
    return jax.named_scope(n) if _SC else _ctx.nullcontext()
XP = 516
NPIN_C = _OPT.get("npin_c", 6)
IMO = _OPT.get("imo", 144)
PLN = _OPT.get("pln", 280)
NPIN_G = _OPT.get("npin_g", 1)


def _slab_rows(j):
    sl = _slabs(j)
    rows = [64 * rho + c0 for rho, c0 in sl]
    return rows + [rows[0]] * (8 - len(rows))


def _kernel(xT_h, wqkv_h, wo_h, uT_h, are_h, aim_h, bre_h, bim_h, cre_h, cim_h, ldt_h, dsk_h, cst_h,
            out_h,
            xT_v, wqkv_v, wo_v, uT_s, par_v, ldt_v, dsk_v, cst_v,
            wt0, wt1, wt2, wt3, wp_s, wo_f, wop_s,
            q_s, k_s, v_s, s_s, o_s,
            pw, gs0, gs1, xk_s, kct_s,
            kuh, yf_s, st_s, dt_s, kop, p_s, tab_s, sems, osem):
    cp_w = [pltpu.make_async_copy(wqkv_h.at[pl.ds(128 * t, 64 if t == 3 else 128), :],
                                  wqkv_v.at[pl.ds(128 * t, 64 if t == 3 else 128), :], sems.at[17 + t]) for t in range(4)]
    cp_x = [pltpu.make_async_copy(xT_h.at[:, pl.ds(512 * b, 512)], xT_v.at[:, pl.ds(512 * b, 512)], sems.at[13 + b])
            for b in range(4)]
    cp_par = [pltpu.make_async_copy(r, par_v.at[i, pl.ds(0, D), :], sems.at[2 + i])
              for i, r in enumerate((are_h, aim_h, bre_h, bim_h, cre_h, cim_h))]
    cp_ldt = pltpu.make_async_copy(ldt_h, ldt_v, sems.at[8])
    cp_dsk = pltpu.make_async_copy(dsk_h, dsk_v, sems.at[9])
    cp_cst = pltpu.make_async_copy(cst_h, cst_v, sems.at[10])
    cp_wo = pltpu.make_async_copy(wo_h, wo_v, sems.at[11])
    cp_u = pltpu.make_async_copy(uT_h, uT_s.at[pl.ds(64, D), :], sems.at[12])
    for c in cp_w:
        c.start()
    cp_x[0].start()
    cp_x[1].start()
    for c in cp_par:
        c.start()
    cp_ldt.start()
    cp_x[2].start()
    cp_x[3].start()
    cp_dsk.start()
    cp_cst.start()
    cp_wo.start()
    cp_u.start()

    nt = (((1,), (1,)), ((), ()))
    tn = (((0,), (0,)), ((), ()))
    PR, PI, ER, EI, MU, ONE = 0, 96, 192, 384, 576, 624

    uT_s[0:64, :] = jnp.zeros((64, SEQ), bf)
    for j in range(16):
        for si, r in enumerate(_slab_rows(j)):
            tab_s[j * 8 + si] = np.int32(r)
    gss = (gs0, gs1)
    for st in range(2):
        for t in range(2):
            gss[st][t, ER + 13 * 12:ER + 16 * 12, :] = jnp.zeros((36, 128), f32)
            gss[st][t, EI + 13 * 12:EI + 16 * 12, :] = jnp.zeros((36, 128), f32)
            gss[st][t, ONE:ONE + 16, :] = jnp.ones((16, 128), f32)
    for rho in range(16):
        xk_s[XP * rho:XP * rho + 64, :] = jnp.zeros((64, 64), f32)
    for lt in range(4):
        yf_s[0, lt, 0:128, :] = jnp.zeros((128, 128), f32)
        yf_s[0, lt, IMO:IMO + 128, :] = jnp.zeros((128, 128), f32)

    wts = (wt0, wt1, wt2, wt3)
    for t in range(4):
        w = 64 if t == 3 else 128
        with _scope('wait_w'):
            cp_w[t].wait()
        wT = wqkv_v[128 * t:128 * t + w, :].T.astype(f32)
        wts[t][0:1344, :] = wT
        wts[t][1344:1352, :] = jnp.zeros((8, w), f32)
        wp_s[0:448, 128 * t:128 * t + w] = wT[0:448].astype(bf)
        wp_s[960:1408, 128 * t:128 * t + w] = wT[896:1344].astype(bf)
        for hh in range(16):
            wp_s[448 + 32 * hh:448 + 32 * hh + 32, 128 * t:128 * t + w] = wts[t][pl.ds(448 + 28 * hh, 32), :].astype(bf)

    def bprep(r0, n):
        sl = pl.ds(r0, n)
        dtc = dt_s[sl, :]
        dt2 = jnp.concatenate([dtc, dtc], axis=1)
        zr = dt2 * par_v[0, sl, :].astype(f32)
        zi = dt2 * par_v[1, sl, :].astype(f32)
        dbr = dt2 * par_v[2, sl, :].astype(f32)
        dbi = dt2 * par_v[3, sl, :].astype(f32)
        cr = par_v[4, sl, :].astype(f32)
        ci_ = par_v[5, sl, :].astype(f32)
        wr_, wi_ = _cmul(cr, ci_, dbr, dbi)
        pw[2, sl, :] = wr_
        pw[3, sl, :] = wi_
        mag = jnp.exp(zr)
        pw[0, sl, :] = mag * jnp.cos(zi)
        pw[1, sl, :] = mag * jnp.sin(zi)

    zpad = jnp.zeros((4, 512), f32)
    opad = jnp.where(lax.broadcasted_iota(jnp.int32, (4, 512), 0) == 0, np.float32(1.0), np.float32(0.0))

    def proj_body(b, carry):
        t0 = pl.multiple_of(b * 512, 512)
        pltpu.make_async_copy(xT_h.at[:, pl.ds(t0, 512)], xT_v.at[:, pl.ds(t0, 512)], sems.at[13 + b]).wait()
        xb = xT_v[:, pl.ds(t0, 512)]
        kT = jnp.dot(wp_s[448:960, :], xb, preferred_element_type=f32)
        qq = jnp.dot(wp_s[0:448, :], xb, preferred_element_type=f32) * np.float32(DH ** -0.5 * LOG2E)
        for hh in range(16):
            q_s[hh, :, pl.ds(t0, 512)] = jnp.concatenate([qq[28 * hh:28 * hh + 28, :], zpad], axis=0).astype(bf)
        vv = jnp.dot(wp_s[960:1408, :], xb, preferred_element_type=f32)
        for hh in range(16):
            v_s[hh, :, pl.ds(t0, 512)] = jnp.concatenate([vv[28 * hh:28 * hh + 28, :], opad], axis=0).astype(bf)
        for g in range(4):
            kg = kT[128 * g:128 * g + 128, :].T
            k_s[4 * g, pl.ds(t0, 512), :] = kg.astype(bf)
            for j in range(1, 4):
                k_s[4 * g + j, pl.ds(t0, 512), :] = pltpu.roll(kg, 128 - 32 * j, 1).astype(bf)
        return carry
    with _scope('proj'):
        lax.fori_loop(0, 4, proj_body, 0)

    for c in cp_par:
        c.wait()
    cp_ldt.wait()
    ldt = ldt_v[...].astype(f32).reshape(1, D)
    dt_row = jnp.exp(ldt).astype(bf).astype(f32)
    dt_s[0:D, :] = jnp.broadcast_to(dt_row, (128, D)).T
    with _scope('wait_rest'):
        cp_cst.wait()
        cp_u.wait()
        cp_dsk.wait()
        cp_wo.wait()
    wo_f[...] = wo_v[...].astype(f32)
    for hh in range(16):
        wop_s[32 * hh:32 * hh + 32, :] = jnp.concatenate(
            [wo_f[28 * hh:28 * hh + 28, :], jnp.zeros((4, D), f32)], axis=0).astype(bf)

    def kgen_prep(b, st):
        d0 = pl.multiple_of(b * 8, 8)
        gs = gss[st]

        def ld_e1():
            return pw[0, pl.ds(d0, 8), :], pw[1, pl.ds(d0, 8), :]

        def ld_w():
            return pw[2, pl.ds(d0, 8), :], pw[3, pl.ds(d0, 8), :]

        def tmp_ld(k):
            return pw[4, 48 * st + 16 * k:48 * st + 16 * k + 8, :], pw[4, 48 * st + 16 * k + 8:48 * st + 16 * k + 16, :]

        def tmp_st(k, v):
            pw[4, 48 * st + 16 * k:48 * st + 16 * k + 8, :] = v[0]
            pw[4, 48 * st + 16 * k + 8:48 * st + 16 * k + 16, :] = v[1]

        def put(base_r, base_i, idx, val):
            for t in range(2):
                sl = slice(128 * t, 128 * t + 128)
                gs[t, base_r + 12 * idx:base_r + 12 * idx + 8, :] = val[0][:, sl]
                gs[t, base_i + 12 * idx:base_i + 12 * idx + 8, :] = val[1][:, sl]

        def get(base_r, base_i, idx):
            return (jnp.concatenate([gs[t, base_r + 12 * idx:base_r + 12 * idx + 8, :] for t in range(2)], axis=1),
                    jnp.concatenate([gs[t, base_i + 12 * idx:base_i + 12 * idx + 8, :] for t in range(2)], axis=1))

        def putm(mi, val):
            for t in range(2):
                sl = slice(128 * t, 128 * t + 128)
                gs[t, MU + 16 * mi:MU + 16 * mi + 8, :] = val[0][:, sl]
                gs[t, MU + 16 * mi + 8:MU + 16 * mi + 16, :] = val[1][:, sl]

        def getm(mi):
            return (jnp.concatenate([gs[t, MU + 16 * mi:MU + 16 * mi + 8, :] for t in range(2)], axis=1),
                    jnp.concatenate([gs[t, MU + 16 * mi + 8:MU + 16 * mi + 16, :] for t in range(2)], axis=1))
        e1, w = ld_e1(), ld_w()
        put(ER, EI, 0, w)
        put(ER, EI, 1, _cmul(*w, *e1))
        e2 = _csq(*e1)
        put(ER, EI, 2, _cmul(*w, *e2))
        tmp_st(0, e2)
        e3 = _cmul(*e2, *e1)
        tmp_st(1, e3)
        yield
        w, e2, e3 = ld_w(), tmp_ld(0), tmp_ld(1)
        put(ER, EI, 3, _cmul(*w, *e3))
        e4 = _csq(*e2)
        tmp_st(2, e4)
        put(ER, EI, 4, _cmul(*w, *e4))
        e6 = _csq(*e3)
        put(ER, EI, 6, _cmul(*w, *e6))
        yield
        e1, w, e3, e4 = ld_e1(), ld_w(), tmp_ld(1), tmp_ld(2)
        put(ER, EI, 5, _cmul(*w, *_cmul(*e4, *e1)))
        put(ER, EI, 7, _cmul(*w, *_cmul(*e4, *e3)))
        e8 = _csq(*e4)
        put(PR, PI, 0, (jnp.ones_like(e8[0]), jnp.zeros_like(e8[0])))
        put(PR, PI, 1, (e8[0], -e8[1]))
        yield
        p1 = get(PR, PI, 1)
        p2 = _csq(*p1)
        put(PR, PI, 2, p2)
        p3 = _cmul(*p2, *p1)
        put(PR, PI, 3, p3)
        p4 = _csq(*p2)
        put(PR, PI, 4, p4)
        put(PR, PI, 5, _cmul(*p4, *p1))
        put(PR, PI, 6, _csq(*p3))
        yield
        p3, p4 = get(PR, PI, 3), get(PR, PI, 4)
        put(PR, PI, 7, _cmul(*p4, *p3))
        m8 = _csq(*p4)
        putm(0, m8)
        m16 = _csq(*m8)
        putm(1, m16)
        m32 = _csq(*m16)
        putm(2, m32)
        yield
        w, e4, m32 = ld_w(), tmp_ld(2), getm(2)
        x512c = _csq(*m32)
        w512 = _cmulc(*w, *x512c)
        put(ER, EI, 8, w512)
        put(ER, EI, 9, _cmul(*w512, *e4))
        x1024c = _csq(*x512c)
        put(ER, EI, 10, _cmulc(*w, *x1024c))
        put(ER, EI, 11, _cmulc(*w, *_cmul(*x1024c, *x512c)))
        put(ER, EI, 12, _cmulc(*w, *_csq(*x1024c)))
        yield

    def kgen_chan(b, i, st):
        d0 = b * 8
        gs = gss[st]
        e2t_r, e2t_i, e1_r, e1_i = [], [], [], []
        for t in range(2):
            b0 = (gs[t, pl.ds(PR + i, 8, stride=12), :], gs[t, pl.ds(PI + i, 8, stride=12), :])

            def mul(mi):
                return (jnp.broadcast_to(gs[t, pl.ds(MU + 16 * mi + i, 1), :], (8, 128)),
                        jnp.broadcast_to(gs[t, pl.ds(MU + 16 * mi + 8 + i, 1), :], (8, 128)))
            mm8, mm16, mm32 = mul(0), mul(1), mul(2)
            b1 = _cmul(*b0, *mm8)
            b2 = _cmul(*b0, *mm16)
            b3 = _cmul(*b1, *mm16)
            b4 = _cmul(*b0, *mm32)
            b5 = _cmul(*b1, *mm32)
            b6 = _cmul(*b2, *mm32)
            b7 = _cmul(*b3, *mm32)
            blks = (b0, b1, b2, b3, b4, b5, b6, b7)
            e2t_r.append(jnp.concatenate([bb[0] for bb in blks], axis=0))
            e2t_i.append(jnp.concatenate([bb[1] for bb in blks], axis=0))
            e1_r.append(gs[t, pl.ds(ER + i, 16, stride=12), :])
            e1_i.append(gs[t, pl.ds(EI + i, 16, stride=12), :])
            if t == 0:
                yield
        lhs = jnp.concatenate(e1_r + e1_i, axis=1).astype(bf)
        rhs = jnp.concatenate(e2t_r + e2t_i, axis=1).astype(bf)
        kc = lax.dot_general(lhs, rhs, nt, preferred_element_type=f32)
        xk_s[pl.ds(64 + d0 + i, 16, stride=XP), :] = kc
        yield

    def kgen_gen(i, st, slot):
        gs = gss[st]
        e2t_r, e2t_i, e1_r, e1_i = [], [], [], []
        for t in range(2):
            b0 = (gs[t, pl.ds(PR + i, 8, stride=12), :], gs[t, pl.ds(PI + i, 8, stride=12), :])

            def mul(mi):
                return (jnp.broadcast_to(gs[t, pl.ds(MU + 16 * mi + i, 1), :], (8, 128)),
                        jnp.broadcast_to(gs[t, pl.ds(MU + 16 * mi + 8 + i, 1), :], (8, 128)))
            mm8, mm16, mm32 = mul(0), mul(1), mul(2)
            b1 = _cmul(*b0, *mm8)
            b2 = _cmul(*b0, *mm16)
            b3 = _cmul(*b1, *mm16)
            b4 = _cmul(*b0, *mm32)
            b5 = _cmul(*b1, *mm32)
            b6 = _cmul(*b2, *mm32)
            b7 = _cmul(*b3, *mm32)
            blks = (b0, b1, b2, b3, b4, b5, b6, b7)
            e2t_r.append(jnp.concatenate([bb[0] for bb in blks], axis=0))
            e2t_i.append(jnp.concatenate([bb[1] for bb in blks], axis=0))
            e1_r.append(gs[t, pl.ds(ER + i, 16, stride=12), :])
            e1_i.append(gs[t, pl.ds(EI + i, 16, stride=12), :])
            if t == 0:
                yield
        kop[slot, 64:80, :] = jnp.concatenate(e1_r + e1_i, axis=1).astype(bf)
        kop[slot, 0:64, :] = jnp.concatenate(e2t_r + e2t_i, axis=1).astype(bf)
        yield

    def kgen_mm(d, slot):
        kc = lax.dot_general(kop[slot, 64:80, :], kop[slot, 0:64, :], nt, preferred_element_type=f32)
        xk_s[pl.ds(64 + d, 16, stride=XP), :] = kc

    def u_fwd(a):
        t0 = pl.multiple_of(a * 128, 128)
        aa = lax.dot_general(cst_v[0], uT_s[:, pl.ds(t0, 128)], nt, preferred_element_type=f32)
        for lt in range(4):
            kuh[1, lt, a, 0:128, :] = aa[0:128, 128 * lt:128 * lt + 128]
            kuh[1, lt, a, IMO:IMO + 128, :] = aa[128:256, 128 * lt:128 * lt + 128]

    def k_tr(rho):
        r0 = pl.multiple_of(rho * XP, 4)
        c0 = pl.multiple_of(rho * 64, 64)
        kct_s[pl.ds(c0, 64), :] = xk_s[pl.ds(r0, 512), :].astype(bf).T

    def k_fwd(j):
        g = jnp.where(j < 2, 1, jnp.where(j < 4, 2, jnp.where(j < 8, 3, 4)))
        win = jnp.concatenate(
            [kct_s[pl.ds(pl.multiple_of(tab_s[j * 8 + si], 16), 16), :] for si in range(8)], axis=0)
        kk = jnp.dot(cst_v[g], win, preferred_element_type=f32)
        for lt in range(4):
            kuh[0, lt, j, 0:128, :] = kk[0:128, 128 * lt:128 * lt + 128]
            kuh[0, lt, j, IMO:IMO + 128, :] = kk[128:256, 128 * lt:128 * lt + 128]

    def conv_pair(unit, p, nsplit):
        lt = unit // 16
        r0 = pl.multiple_of((unit % 16) * 8, 8)
        a0 = 2 * p
        a1 = 2 * p + 1
        ar0 = ai0 = ar1 = ai1 = None
        uprev = None
        cuts = set(int(round((a1 + 1) * k / nsplit)) for k in range(1, nsplit))
        for j in range(a1 + 1):
            if j in cuts:
                yield
            kr = kuh[0, lt, j, pl.ds(r0, 8), :]
            ki = kuh[0, lt, j, pl.ds(IMO + r0, 8), :]
            m1 = a1 - j
            if uprev is None:
                u1 = (kuh[1, lt, m1, pl.ds(r0, 8), :], kuh[1, lt, m1, pl.ds(IMO + r0, 8), :])
            else:
                u1 = uprev
            tr = kr * u1[0] - ki * u1[1]
            ti = kr * u1[1] + ki * u1[0]
            ar1 = tr if ar1 is None else ar1 + tr
            ai1 = ti if ai1 is None else ai1 + ti
            m0 = a0 - j
            if m0 >= 0:
                u0 = (kuh[1, lt, m0, pl.ds(r0, 8), :], kuh[1, lt, m0, pl.ds(IMO + r0, 8), :])
                tr = kr * u0[0] - ki * u0[1]
                ti = kr * u0[1] + ki * u0[0]
                ar0 = tr if ar0 is None else ar0 + tr
                ai0 = ti if ai0 is None else ai0 + ti
                uprev = u0
        for a, (yr, yi) in ((a0, (ar0, ai0)), (a1, (ar1, ai1))):
            yf_s[a + 1, lt, pl.ds(r0, 8), :] = yr
            yf_s[a + 1, lt, pl.ds(IMO + r0, 8), :] = yi
        yield

    cim = jnp.concatenate([cst_v[5, 0:128, :], cst_v[5, 128:256, :]], axis=1)
    sgn = jnp.where(lax.broadcasted_iota(jnp.int32, (128, 128), 0) % 2 == 0, np.float32(1.0), np.float32(-1.0))

    def inverse(a):
        t0 = pl.multiple_of(a * 128, 128)
        parts = []
        for lt in range(4):
            yr = yf_s[a + 1, lt, 0:128, :] - sgn * yf_s[a, lt, IMO:IMO + 128, :]
            yi = yf_s[a + 1, lt, IMO:IMO + 128, :] + sgn * yf_s[a, lt, 0:128, :]
            parts.append(jnp.concatenate([yr, yi], axis=0).astype(bf))
        yy = jnp.concatenate(parts, axis=1)
        y = jnp.dot(cim, yy, preferred_element_type=f32).astype(bf)
        st_s[pl.ds(t0, 128), 448:512] = y[:, 64:128]
        st_s[pl.ds(t0, 128), 512:896] = y[:, 128:512]

    NB = NQB * H
    NC = SEQ // CK

    def q_of(i):
        qb = i // H
        h = i % H
        q0 = pl.multiple_of(qb * BQ, BQ)
        return q_s[h, :, pl.ds(q0, BQ)], h

    def pv_chunk(h, c, m, acc):
        s = s_s[pl.ds(c * CK, CK), :]
        p = jnp.exp2(s - m).astype(bf)
        o = jnp.dot(v_s[h, :, pl.ds(c * CK, CK)], p, preferred_element_type=f32)
        return o if acc is None else acc + o

    def p_make(c, m):
        s = s_s[pl.ds(c * CK, CK), :]
        p_s[c % 2, 0:CK, :] = jnp.exp2(s - m).astype(bf)

    def p_make_half(c, m, hf):
        s = s_s[pl.ds(c * CK + hf * (CK // 2), CK // 2), :]
        p_s[c % 2, hf * (CK // 2):(hf + 1) * (CK // 2), :] = jnp.exp2(s - m).astype(bf)

    def pv_mm(h, c, acc):
        o = jnp.dot(v_s[h, :, pl.ds(c * CK, CK)], p_s[c % 2, 0:CK, :], preferred_element_type=f32)
        return o if acc is None else acc + o

    def qk_mm(h, qm, c):
        return jnp.dot(k_s[h, pl.ds(c * CK, CK), 0:32], qm, preferred_element_type=f32)

    def qk_fin(s, c, mrun, pins=None, tasks=()):
        s_s[pl.ds(c * CK, CK), :] = s
        mm = jnp.max(s.reshape(CK // 8, 8, BQ), axis=0)
        if pins is not None:
            groups = pins if isinstance(pins, list) else [pins]
            events = []
            for gi, (pin_store, npin, pinned) in enumerate(groups):
                for k in range(npin):
                    g = (k + 1) * (CK // 8) // npin - 1 if npin > 1 else _OPT.get("pin1_g", 7)
                    if gi > 0:
                        g = (_OPT.get("pk0", 3), _OPT.get("pk1", 11))[k]
                    events.append((g, gi))
            for g, gi in sorted(events):
                pin_store, npin, pinned = groups[gi]
                pin_store(s[8 * g:8 * g + 8, 0:128])
                for t in pinned:
                    next(t, None)
            for pin_store, npin, pinned in groups:
                for t in pinned:
                    for _ in t:
                        pass
        for t in tasks:
            for _ in t:
                pass
        return mm if mrun is None else jnp.maximum(mrun, mm)

    qm0, h0 = q_of(0)
    mrun = None
    for c in range(NC):
        mrun = qk_fin(qk_mm(0, qm0, c), c, mrun)

    cfg = {}

    PSTPIN = _OPT.get('pstpin', [-1, -1])

    def att_step(i, mrun_prev, extra, pst=False):
        m_cur = jnp.max(mrun_prev, axis=0, keepdims=True)
        inext = jnp.minimum(i + 1, NB - 1)
        qm, hn = q_of(inext)
        qb = i // H
        h = i % H
        mrun = None
        acc = None
        state = {}
        for c in range(NC):
            pre = None
            if extra is not None and _OPT.get("gmode", 0) == 2:
                pre = extra(i, c, state)
                for t in state.pop('pre', []):
                    for _ in t:
                        pass
            if pst:
                if c == 0:
                    p_make(0, m_cur)
                acc = pv_mm(h, c, acc)
                s = qk_mm(hn, qm, c)
                if c + 1 < NC:
                    dzp = pl.multiple_of(CK + opaque(i, 13) * 16, 16)
                    for hf in range(2):
                        if PSTPIN[hf] >= 0:
                            g = PSTPIN[hf]
                            p_s[(c + 1) % 2, pl.ds(dzp, 16), 0:128] = jnp.concatenate([s[8 * g:8 * g + 8, 0:128]] * 2, axis=0).astype(bf)
                        p_make_half(c + 1, m_cur, hf)
            elif c < cfg['nqf']:
                s = qk_mm(hn, qm, c)
                acc = pv_chunk(h, c, m_cur, acc)
            else:
                acc = pv_chunk(h, c, m_cur, acc)
                s = qk_mm(hn, qm, c)
            pins, tasks = (None, ()) if extra is None else (pre if pre is not None else extra(i, c, state))
            mrun = qk_fin(s, c, mrun, pins, tasks)
        inv = 1.0 / acc[28:29, :]
        q0 = pl.multiple_of(qb * BQ, BQ)
        o_s[h, :, pl.ds(q0, BQ)] = (acc * inv).astype(bf)
        return mrun


    def run(lo, hi, extra, mrun, name=''):
        pst = name in _OPT.get('pst', [])
        UN = _OPT.get('uns', {}).get(name, 1)
        cfg['nqf'] = _OPT.get('nqfs', {}).get(name, 0)

        def body(t, mrun):
            for u in range(UN):
                mrun = att_step(t * UN + u, mrun, extra, pst)
            return mrun
        return lax.fori_loop(lo // UN, hi // UN, body, mrun)

    def opaque(i, k):
        return (i * k) >> 12

    def fn_task(fn, *a):
        def g():
            fn(*a)
            yield
        return g()

    I_G, I_T, I_KF, I_C, I_I = 4, 32, 36, 40, 56

    def ex_P(i, c, state):
        tasks = []
        if c % 4 == 1:
            tasks.append(fn_task(u_fwd, i * 4 + c // 4))
        if _OPT.get("ppin", 1) == 0:
            if c in (0, 8):
                r0 = pl.multiple_of(i * 112 + (0 if c == 0 else 48), 16)
                tasks.append(fn_task(bprep, r0, 48 if c == 0 else 64))
            return None, tasks
        if c % 2 == 0 and c < 14:
            r0 = pl.multiple_of(i * 112 + 16 * (c // 2), 16)
            dzq = pl.multiple_of(D + opaque(i, 9) * 16, 16)

            def pin_store(v):
                dt_s[pl.ds(dzq, 8), :] = v
                par_v[0, pl.ds(dzq, 16), 0:128] = jnp.concatenate([v, v], axis=0).astype(bf)
            return (pin_store, 1, [fn_task(bprep, r0, 16)]), tasks
        return None, tasks

    def ex_G(i, c, state):
        j = i - I_G
        st = c // 8
        dz = pl.multiple_of(448 + opaque(i, 9) * 8, 8)

        def pin_store(v):
            pw[4, pl.ds(dz, 8), 0:128] = v
        tasks = [kgen_chan(2 * j + st, c % 8, st)]
        pinned = []
        if c % 8 == 0:
            nb = 2 * j + 1 if st == 0 else jnp.minimum(2 * j + 2, D // 8 - 1)
            state['prep'] = kgen_prep(nb, 1 - st)
        if c % 8 < 6:
            pinned.append(fn_task(next, state['prep']))
        mode = _OPT.get("gmode", 0)
        if mode == 1:
            dz2 = pl.multiple_of(ONE + opaque(i, 11) * 8, 8)

            def pin_store2(v):
                gss[st][0, pl.ds(dz2, 8), :] = v
            groups = [(pin_store, NPIN_G, pinned)] if pinned else []
            groups.append((pin_store2, 2, tasks))
            return groups, []
        if mode == 3:
            dz2 = pl.multiple_of(ONE + opaque(i, 11) * 8, 8)

            def pin_store2(v):
                gss[st][0, pl.ds(dz2, 8), :] = v
            tasks = []
            if c > 0:
                cp = c - 1
                tasks.append(fn_task(kgen_mm, (2 * j + cp // 8) * 8 + cp % 8, cp % 2))
            gen = kgen_gen(c % 8, st, c % 2)
            if c == NC - 1:
                def last(gen=gen):
                    for _ in gen:
                        pass
                    kgen_mm((2 * j + 1) * 8 + 7, c % 2)
                    yield
                tasks.append(last())
                gen = None
            groups = [(pin_store, NPIN_G, pinned)] if pinned else []
            if gen is not None:
                if _OPT.get("gpin", 1):
                    groups.append((pin_store2, 2, [gen]))
                else:
                    tasks.append(gen)
            return (groups if groups else None), tasks
        if mode == 2:
            state['pre'] = tasks
            tasks = []
        if NPIN_G == 0 or not pinned:
            return None, pinned + tasks
        return (pin_store, NPIN_G, pinned), tasks

    def ex_T(i, c, state):
        if c % 4 == 1:
            return None, [fn_task(k_tr, (i - I_T) * 4 + c // 4)]
        return None, []

    def ex_KF(i, c, state):
        if c % 4 == 1:
            return None, [fn_task(k_fwd, (i - I_KF) * 4 + c // 4)]
        return None, []

    def ex_C(i, c, state):
        dz = 16 + opaque(i, 9)

        def pin_store(v):
            kuh[0, 0, dz, 0:8, :] = v
        ub = (i - I_C) * 4 + c // 4
        pp = c % 4
        return (pin_store, NPIN_C, [conv_pair(ub, pp, NPIN_C), conv_pair(ub, 7 - pp, NPIN_C)]), []

    def ex_I(i, c, state):
        if c % 8 == 2:
            return None, [fn_task(inverse, (i - I_I) * 2 + c // 8)]
        return None, []

    out_cps = []

    def outproj_body(qb, carry):
        q0 = pl.multiple_of(qb * BQ, BQ)
        oT = o_s[:, :, pl.ds(q0, BQ)].reshape(512, BQ)
        ya = lax.dot_general(oT, wop_s[...], tn, preferred_element_type=f32)
        st_s[pl.ds(q0, BQ), 0:448] = ya.astype(bf)
        pltpu.make_async_copy(st_s.at[pl.ds(q0, BQ), :], out_h.at[0, pl.ds(q0, BQ), :], osem.at[qb]).start()
        return carry

    with _scope('P'):
        mrun = run(0, I_G, ex_P, mrun, 'P')
    for _ in kgen_prep(0, 0):
        pass
    with _scope('G'):
        mrun = run(I_G, I_T, ex_G, mrun, 'G')
    with _scope('T'):
        mrun = run(I_T, I_KF, ex_T, mrun, 'T')
    with _scope('KF'):
        mrun = run(I_KF, I_C, ex_KF, mrun, 'KF')
    dsk = jnp.concatenate([jnp.zeros((1, 64), f32), dsk_v[...].astype(f32).reshape(1, D)], axis=1)
    for lt in range(4):
        kuh[0, lt, 0, 0:128, :] = kuh[0, lt, 0, 0:128, :] + dsk[:, 128 * lt:128 * lt + 128]
    with _scope('C'):
        mrun = run(I_C, I_I, ex_C, mrun, 'C')
    with _scope('I'):
        mrun = run(I_I, NB, ex_I, mrun, 'I')
    with _scope('outproj'):
        lax.fori_loop(0, NQB, outproj_body, 0)
    with _scope('outwait'):
      for qb in range(NQB):
        pltpu.make_async_copy(st_s.at[pl.ds(qb * BQ, BQ), :], out_h.at[0, pl.ds(qb * BQ, BQ), :], osem.at[qb]).wait()


@jax.jit
def pallas_concat_heads__mha_block__ssm_conv_s4__prompt_kernel(
        A_x, A_wqkv, A_wo, B_u, B_A_re, B_A_im, B_B_re, B_B_im, B_C_re, B_C_im, B_log_dt, B_Dskip):
    hbm = pl.BlockSpec(memory_space=pltpu.HBM)
    scratch = [
        pltpu.VMEM((D, SEQ), bf),
        pltpu.VMEM((D, 3 * D), bf),
        pltpu.VMEM((D, D), bf),
        pltpu.VMEM((512, SEQ), bf),
        pltpu.VMEM((6, D + 16, NST), bf),
        pltpu.VMEM((D,), bf),
        pltpu.VMEM((D,), bf),
        pltpu.VMEM((6, 256, 128), bf),
        pltpu.VMEM((1352, 128), f32), pltpu.VMEM((1352, 128), f32),
        pltpu.VMEM((1352, 128), f32), pltpu.VMEM((1352, 64), f32),
        pltpu.VMEM((1408, D), bf),
        pltpu.VMEM((D, D), f32),
        pltpu.VMEM((512, D), bf),
        pltpu.VMEM((16, 32, SEQ), bf),
        pltpu.VMEM((16, SEQ, 128), bf),
        pltpu.VMEM((16, 32, SEQ), bf),
        pltpu.VMEM((SEQ, BQ), f32),
        pltpu.VMEM((16, 32, SEQ), bf),
        pltpu.VMEM((5, 456, NST), f32),
        pltpu.VMEM((2, 640, 128), f32), pltpu.VMEM((2, 640, 128), f32),
        pltpu.VMEM((XP * 16, 64), f32),
        pltpu.VMEM((1024, 512), bf),
        pltpu.VMEM((2, 4, 17, PLN, 128), f32),
        pltpu.VMEM((17, 4, PLN, 128), f32),
        pltpu.VMEM((SEQ, 896), bf),
        pltpu.VMEM((D + 16, 128), f32),
        pltpu.VMEM((2, 80, 512), bf),
        pltpu.VMEM((2, CK + 16, BQ), bf),
        pltpu.SMEM((128,), jnp.int32),
        pltpu.SemaphoreType.DMA((21,)),
        pltpu.SemaphoreType.DMA((4,)),
    ]
    c = lambda a: pltpu.with_memory_space_constraint(a, pltpu.HBM)
    xT = jnp.transpose(A_x[0])
    uT = jnp.transpose(B_u[0])
    args = [c(a) for a in (xT, A_wqkv, A_wo, uT, B_A_re, B_A_im, B_B_re, B_B_im, B_C_re, B_C_im,
                           B_log_dt, B_Dskip, jnp.asarray(_CONSTS))]
    return pl.pallas_call(
        _kernel,
        out_shape=jax.ShapeDtypeStruct((1, SEQ, 2 * D), bf),
        in_specs=[hbm] * 13,
        out_specs=hbm,
        scratch_shapes=scratch,
        compiler_params=pltpu.CompilerParams(vmem_limit_bytes=110 * 2 ** 20, flags=_FLAGS),
    )(*args)
```

```python
import functools
import numpy as np
import ml_dtypes
import jax
import jax.numpy as jnp
from jax import lax
from jax.experimental import pallas as pl
from jax.experimental.pallas import tpu as pltpu

bf = jnp.bfloat16
f32 = jnp.float32

SEQ = 2048
D = 448
H = 16
DH = 28
NST = 256
BQ = 512
CK = 128
NQB = SEQ // BQ
LOG2E = 1.4426950408889634

_L1 = np.array([0, 1, 2, 3, 4, 5, 6, 7, 512, 516, 1024, 1536, 2048])


def _slabs(j):
    if j < 2:
        return [(r, 16 * j) for r in range(8)]
    if j < 4:
        return [(r, 16 * j) for r in (0, 2, 4, 6)] + [(0, 48) if j == 2 else (8, 0)]
    if j < 8:
        return [(8, 16 * (j - 4)), (9, 16 * (j - 4))] + [(8, 16 * (j - 3)) if j < 7 else (10, 0)]
    if j < 12:
        return [(10, 16 * (j - 8))] + [(10, 16 * (j - 7)) if j < 11 else (11, 0)]
    return [(11, 16 * (j - 12))] + [(11, 16 * (j - 11)) if j < 15 else (12, 0)]


def _group(j):
    return 0 if j < 2 else 1 if j < 4 else 2 if j < 8 else 3


def _make_consts():
    k = np.arange(128)[:, None]
    n = np.arange(128)[None, :]
    ang = np.pi * (2 * k + 1) * n / 256.0
    ct = np.concatenate([np.cos(ang), -np.sin(ang)], 0)
    n2 = (128 + np.arange(128))[:, None]
    k2 = np.arange(128)[None, :]
    ang2 = np.pi * (2 * k2 + 1) * n2 / 256.0
    ci = np.concatenate([np.cos(ang2), -np.sin(ang2)], 1) / 128.0
    n2 = np.arange(128)[:, None]
    ang2 = np.pi * (2 * k2 + 1) * n2 / 256.0
    ci = np.concatenate([np.cos(ang2), -np.sin(ang2)], 1) / 128.0
    out = np.zeros((6, 256, 128), np.float64)
    out[0] = ct
    for g, j in enumerate((0, 2, 4, 8)):
        pos = {}
        sl = _slabs(j)
        for si, (rho, c0) in enumerate(sl):
            for cc in range(16):
                pos.setdefault(int(_L1[rho] + 8 * (c0 + cc)), si * 16 + cc)
        m = np.zeros((256, 128))
        for nn in range(128):
            lr = int(np.float32(128 * j + nn).astype(ml_dtypes.bfloat16).astype(np.float32))
            m[:, pos[lr]] += ct[:, nn]
        out[g + 1] = m
    out[5, 0:128] = ci[:, 0:128]
    out[5, 128:256] = ci[:, 128:256]
    return out.astype(np.float32).astype(ml_dtypes.bfloat16)


_CONSTS = _make_consts()
_WIN = (128, 80, 48, 32)


def _cmul(ar, ai, br, bi):
    return ar * br - ai * bi, ar * bi + ai * br


def _cmulc(ar, ai, br, bi):
    return ar * br + ai * bi, ai * br - ar * bi


def _csq(ar, ai):
    return ar * ar - ai * ai, (ar + ar) * ai


_FLAGS = None
_OPT = OPQ
import contextlib as _ctx
_SC = _OPT.get('scopes', False)
def _scope(n):
    return jax.named_scope(n) if _SC else _ctx.nullcontext()
XP = 516
NPIN_C = _OPT.get("npin_c", 6)
IMO = _OPT.get("imo", 144)
PLN = _OPT.get("pln", 280)
NPIN_G = _OPT.get("npin_g", 1)


def _sincos(x):
    kf = jnp.round(x * np.float32(2.0 / np.pi))
    ki = kf.astype(jnp.int32)
    r = x - kf * np.float32(1.5703125)
    r = r - kf * np.float32(4.837512969970703125e-4)
    r = r - kf * np.float32(7.54978995489188216e-8)
    r2 = r * r
    s = r + r * r2 * (np.float32(-1.6666654611e-1) + r2 * (np.float32(8.3321608736e-3) + r2 * np.float32(-1.9515295891e-4)))
    c = (np.float32(1.0) - np.float32(0.5) * r2) + r2 * r2 * (
        np.float32(4.166664568298827e-2) + r2 * (np.float32(-1.388731625493765e-3) + r2 * np.float32(2.443315711809948e-5)))
    swap = (ki & 1) == 1
    sb = jnp.where(swap, c, s)
    cb = jnp.where(swap, s, c)
    sn = jnp.where((ki & 2) != 0, -sb, sb)
    cs = jnp.where(((ki + 1) & 2) != 0, -cb, cb)
    return sn, cs


def _slab_rows(j):
    sl = _slabs(j)
    rows = [64 * rho + c0 for rho, c0 in sl]
    return rows + [rows[0]] * (8 - len(rows))


def _kernel(xT_h, wqkv_h, wo_h, uT_h, are_h, aim_h, bre_h, bim_h, cre_h, cim_h, ldt_h, dsk_h, cst_h,
            out_h,
            xT_v, wqkv_v, wo_v, uT_s, par_v, ldt_v, dsk_v, cst_v,
            wt0, wt1, wt2, wt3, wp_s, wo_f, wop_s,
            q_s, k_s, v_s, s_s, o_s,
            pw, gs0, gs1, xk_s, kct_s,
            kuh, yf_s, st_s, dt_s, kop, p_s, mr_s, tab_s, sems, osem):
    cp_w = [pltpu.make_async_copy(wqkv_h.at[pl.ds(128 * t, 64 if t == 3 else 128), :],
                                  wqkv_v.at[pl.ds(128 * t, 64 if t == 3 else 128), :], sems.at[17 + t]) for t in range(4)]
    cp_x = [pltpu.make_async_copy(xT_h.at[:, pl.ds(512 * b, 512)], xT_v.at[:, pl.ds(512 * b, 512)], sems.at[13 + b])
            for b in range(4)]
    cp_par = [pltpu.make_async_copy(r, par_v.at[i, pl.ds(0, D), :], sems.at[2 + i])
              for i, r in enumerate((are_h, aim_h, bre_h, bim_h, cre_h, cim_h))]
    cp_ldt = pltpu.make_async_copy(ldt_h, ldt_v, sems.at[8])
    cp_dsk = pltpu.make_async_copy(dsk_h, dsk_v, sems.at[9])
    cp_cst = pltpu.make_async_copy(cst_h, cst_v, sems.at[10])
    cp_wo = pltpu.make_async_copy(wo_h, wo_v, sems.at[11])
    cp_u = pltpu.make_async_copy(uT_h, uT_s.at[pl.ds(64, D), :], sems.at[12])
    for c in cp_w:
        c.start()
    cp_x[0].start()
    cp_x[1].start()
    for c in cp_par:
        c.start()
    cp_ldt.start()
    cp_x[2].start()
    cp_x[3].start()
    cp_dsk.start()
    cp_cst.start()
    cp_wo.start()
    cp_u.start()

    nt = (((1,), (1,)), ((), ()))
    tn = (((0,), (0,)), ((), ()))
    PR, PI, ER, EI, MU, ONE = 0, 96, 192, 384, 576, 624

    uT_s[0:64, :] = jnp.zeros((64, SEQ), bf)
    for j in range(16):
        for si, r in enumerate(_slab_rows(j)):
            tab_s[j * 8 + si] = np.int32(r)
    gss = (gs0, gs1)
    for st in range(2):
        for t in range(2):
            gss[st][t, ER + 13 * 12:ER + 16 * 12, :] = jnp.zeros((36, 128), f32)
            gss[st][t, EI + 13 * 12:EI + 16 * 12, :] = jnp.zeros((36, 128), f32)
            gss[st][t, ONE:ONE + 16, :] = jnp.ones((16, 128), f32)
    for rho in range(16):
        xk_s[XP * rho:XP * rho + 64, :] = jnp.zeros((64, 64), f32)
    for lt in range(4):
        yf_s[0, lt, 0:128, :] = jnp.zeros((128, 128), f32)
        yf_s[0, lt, IMO:IMO + 128, :] = jnp.zeros((128, 128), f32)

    wts = (wt0, wt1, wt2, wt3)
    for t in range(4):
        w = 64 if t == 3 else 128
        with _scope('wait_w'):
            cp_w[t].wait()
        wT = wqkv_v[128 * t:128 * t + w, :].T.astype(f32)
        wts[t][0:1344, :] = wT
        wts[t][1344:1352, :] = jnp.zeros((8, w), f32)
        wp_s[0:448, 128 * t:128 * t + w] = wT[0:448].astype(bf)
        wp_s[960:1408, 128 * t:128 * t + w] = wT[896:1344].astype(bf)
        for hh in range(16):
            wp_s[448 + 32 * hh:448 + 32 * hh + 32, 128 * t:128 * t + w] = wts[t][pl.ds(448 + 28 * hh, 32), :].astype(bf)

    def bprep(r0, n, fast=False):
        sl = pl.ds(r0, n)
        dtc = dt_s[sl, :]
        dt2 = jnp.concatenate([dtc, dtc], axis=1)
        zr = dt2 * par_v[0, sl, :].astype(f32)
        zi = dt2 * par_v[1, sl, :].astype(f32)
        dbr = dt2 * par_v[2, sl, :].astype(f32)
        dbi = dt2 * par_v[3, sl, :].astype(f32)
        cr = par_v[4, sl, :].astype(f32)
        ci_ = par_v[5, sl, :].astype(f32)
        wr_, wi_ = _cmul(cr, ci_, dbr, dbi)
        pw[2, sl, :] = wr_
        pw[3, sl, :] = wi_
        mag = jnp.exp(zr)
        if fast:
            sn, cs = _sincos(zi)
        else:
            sn, cs = jnp.sin(zi), jnp.cos(zi)
        pw[0, sl, :] = mag * cs
        pw[1, sl, :] = mag * sn

    zpad = jnp.zeros((4, 512), f32)
    opad = jnp.where(lax.broadcasted_iota(jnp.int32, (4, 512), 0) == 0, np.float32(1.0), np.float32(0.0))

    def proj_body(b, carry):
        t0 = pl.multiple_of(b * 512, 512)
        pltpu.make_async_copy(xT_h.at[:, pl.ds(t0, 512)], xT_v.at[:, pl.ds(t0, 512)], sems.at[13 + b]).wait()
        xb = xT_v[:, pl.ds(t0, 512)]
        kT = jnp.dot(wp_s[448:960, :], xb, preferred_element_type=f32)
        qq = jnp.dot(wp_s[0:448, :], xb, preferred_element_type=f32) * np.float32(DH ** -0.5 * LOG2E)
        for hh in range(16):
            q_s[hh, :, pl.ds(t0, 512)] = jnp.concatenate([qq[28 * hh:28 * hh + 28, :], zpad], axis=0).astype(bf)
        vv = jnp.dot(wp_s[960:1408, :], xb, preferred_element_type=f32)
        for hh in range(16):
            v_s[hh, :, pl.ds(t0, 512)] = jnp.concatenate([vv[28 * hh:28 * hh + 28, :], opad], axis=0).astype(bf)
        for g in range(4):
            kg = kT[128 * g:128 * g + 128, :].T
            k_s[4 * g, pl.ds(t0, 512), :] = kg.astype(bf)
            for j in range(1, 4):
                k_s[4 * g + j, pl.ds(t0, 512), :] = pltpu.roll(kg, 128 - 32 * j, 1).astype(bf)
        return carry
    with _scope('proj'):
        lax.fori_loop(0, 4, proj_body, 0)

    for c in cp_par:
        c.wait()
    cp_ldt.wait()
    ldt = ldt_v[...].astype(f32).reshape(1, D)
    dt_row = jnp.exp(ldt).astype(bf).astype(f32)
    dt_s[0:D, :] = jnp.broadcast_to(dt_row, (128, D)).T
    with _scope('wait_rest'):
        cp_cst.wait()
        cp_u.wait()
        cp_dsk.wait()
        cp_wo.wait()
    wo_f[...] = wo_v[...].astype(f32)
    for hh in range(16):
        wop_s[32 * hh:32 * hh + 32, :] = jnp.concatenate(
            [wo_f[28 * hh:28 * hh + 28, :], jnp.zeros((4, D), f32)], axis=0).astype(bf)

    def kgen_prep(b, st, tiles=(0, 1)):
        d0 = pl.multiple_of(b * 8, 8)
        gs = gss[st]
        ls = slice(128 * tiles[0], 128 * tiles[-1] + 128)

        def ld_e1():
            return pw[0, pl.ds(d0, 8), ls], pw[1, pl.ds(d0, 8), ls]

        def ld_w():
            return pw[2, pl.ds(d0, 8), ls], pw[3, pl.ds(d0, 8), ls]

        def tmp_ld(k):
            return pw[4, 48 * st + 16 * k:48 * st + 16 * k + 8, ls], pw[4, 48 * st + 16 * k + 8:48 * st + 16 * k + 16, ls]

        def tmp_st(k, v):
            pw[4, 48 * st + 16 * k:48 * st + 16 * k + 8, ls] = v[0]
            pw[4, 48 * st + 16 * k + 8:48 * st + 16 * k + 16, ls] = v[1]

        def put(base_r, base_i, idx, val):
            for n, t in enumerate(tiles):
                sl = slice(128 * n, 128 * n + 128)
                gs[t, base_r + 12 * idx:base_r + 12 * idx + 8, :] = val[0][:, sl]
                gs[t, base_i + 12 * idx:base_i + 12 * idx + 8, :] = val[1][:, sl]

        def get(base_r, base_i, idx):
            return (jnp.concatenate([gs[t, base_r + 12 * idx:base_r + 12 * idx + 8, :] for t in tiles], axis=1),
                    jnp.concatenate([gs[t, base_i + 12 * idx:base_i + 12 * idx + 8, :] for t in tiles], axis=1))

        def putm(mi, val):
            for n, t in enumerate(tiles):
                sl = slice(128 * n, 128 * n + 128)
                gs[t, MU + 16 * mi:MU + 16 * mi + 8, :] = val[0][:, sl]
                gs[t, MU + 16 * mi + 8:MU + 16 * mi + 16, :] = val[1][:, sl]

        def getm(mi):
            return (jnp.concatenate([gs[t, MU + 16 * mi:MU + 16 * mi + 8, :] for t in tiles], axis=1),
                    jnp.concatenate([gs[t, MU + 16 * mi + 8:MU + 16 * mi + 16, :] for t in tiles], axis=1))
        e1, w = ld_e1(), ld_w()
        put(ER, EI, 0, w)
        put(ER, EI, 1, _cmul(*w, *e1))
        e2 = _csq(*e1)
        put(ER, EI, 2, _cmul(*w, *e2))
        tmp_st(0, e2)
        e3 = _cmul(*e2, *e1)
        tmp_st(1, e3)
        yield
        w, e2, e3 = ld_w(), tmp_ld(0), tmp_ld(1)
        put(ER, EI, 3, _cmul(*w, *e3))
        e4 = _csq(*e2)
        tmp_st(2, e4)
        put(ER, EI, 4, _cmul(*w, *e4))
        e6 = _csq(*e3)
        put(ER, EI, 6, _cmul(*w, *e6))
        yield
        e1, w, e3, e4 = ld_e1(), ld_w(), tmp_ld(1), tmp_ld(2)
        put(ER, EI, 5, _cmul(*w, *_cmul(*e4, *e1)))
        put(ER, EI, 7, _cmul(*w, *_cmul(*e4, *e3)))
        e8 = _csq(*e4)
        put(PR, PI, 0, (jnp.ones_like(e8[0]), jnp.zeros_like(e8[0])))
        put(PR, PI, 1, (e8[0], -e8[1]))
        yield
        p1 = get(PR, PI, 1)
        p2 = _csq(*p1)
        put(PR, PI, 2, p2)
        p3 = _cmul(*p2, *p1)
        put(PR, PI, 3, p3)
        p4 = _csq(*p2)
        put(PR, PI, 4, p4)
        put(PR, PI, 5, _cmul(*p4, *p1))
        put(PR, PI, 6, _csq(*p3))
        yield
        p3, p4 = get(PR, PI, 3), get(PR, PI, 4)
        put(PR, PI, 7, _cmul(*p4, *p3))
        m8 = _csq(*p4)
        putm(0, m8)
        m16 = _csq(*m8)
        putm(1, m16)
        m32 = _csq(*m16)
        putm(2, m32)
        yield
        w, e4, m32 = ld_w(), tmp_ld(2), getm(2)
        x512c = _csq(*m32)
        w512 = _cmulc(*w, *x512c)
        put(ER, EI, 8, w512)
        put(ER, EI, 9, _cmul(*w512, *e4))
        x1024c = _csq(*x512c)
        put(ER, EI, 10, _cmulc(*w, *x1024c))
        put(ER, EI, 11, _cmulc(*w, *_cmul(*x1024c, *x512c)))
        put(ER, EI, 12, _cmulc(*w, *_csq(*x1024c)))
        yield

    def kgen_chan(b, i, st):
        d0 = b * 8
        gs = gss[st]
        e2t_r, e2t_i, e1_r, e1_i = [], [], [], []
        for t in range(2):
            b0 = (gs[t, pl.ds(PR + i, 8, stride=12), :], gs[t, pl.ds(PI + i, 8, stride=12), :])

            def mul(mi):
                return (jnp.broadcast_to(gs[t, pl.ds(MU + 16 * mi + i, 1), :], (8, 128)),
                        jnp.broadcast_to(gs[t, pl.ds(MU + 16 * mi + 8 + i, 1), :], (8, 128)))
            mm8, mm16, mm32 = mul(0), mul(1), mul(2)
            b1 = _cmul(*b0, *mm8)
            b2 = _cmul(*b0, *mm16)
            b3 = _cmul(*b1, *mm16)
            b4 = _cmul(*b0, *mm32)
            b5 = _cmul(*b1, *mm32)
            b6 = _cmul(*b2, *mm32)
            b7 = _cmul(*b3, *mm32)
            blks = (b0, b1, b2, b3, b4, b5, b6, b7)
            e2t_r.append(jnp.concatenate([bb[0] for bb in blks], axis=0))
            e2t_i.append(jnp.concatenate([bb[1] for bb in blks], axis=0))
            e1_r.append(gs[t, pl.ds(ER + i, 16, stride=12), :])
            e1_i.append(gs[t, pl.ds(EI + i, 16, stride=12), :])
            if t == 0:
                yield
        lhs = jnp.concatenate(e1_r + e1_i, axis=1).astype(bf)
        rhs = jnp.concatenate(e2t_r + e2t_i, axis=1).astype(bf)
        kc = lax.dot_general(lhs, rhs, nt, preferred_element_type=f32)
        xk_s[pl.ds(64 + d0 + i, 16, stride=XP), :] = kc
        yield

    def kgen_gen(i, st, slot):
        gs = gss[st]
        e2t_r, e2t_i, e1_r, e1_i = [], [], [], []
        for t in range(2):
            b0 = (gs[t, pl.ds(PR + i, 8, stride=12), :], gs[t, pl.ds(PI + i, 8, stride=12), :])

            def mul(mi):
                return (jnp.broadcast_to(gs[t, pl.ds(MU + 16 * mi + i, 1), :], (8, 128)),
                        jnp.broadcast_to(gs[t, pl.ds(MU + 16 * mi + 8 + i, 1), :], (8, 128)))
            mm8, mm16, mm32 = mul(0), mul(1), mul(2)
            b1 = _cmul(*b0, *mm8)
            b2 = _cmul(*b0, *mm16)
            b3 = _cmul(*b1, *mm16)
            b4 = _cmul(*b0, *mm32)
            b5 = _cmul(*b1, *mm32)
            b6 = _cmul(*b2, *mm32)
            b7 = _cmul(*b3, *mm32)
            blks = (b0, b1, b2, b3, b4, b5, b6, b7)
            e2t_r.append(jnp.concatenate([bb[0] for bb in blks], axis=0))
            e2t_i.append(jnp.concatenate([bb[1] for bb in blks], axis=0))
            e1_r.append(gs[t, pl.ds(ER + i, 16, stride=12), :])
            e1_i.append(gs[t, pl.ds(EI + i, 16, stride=12), :])
            if t == 0:
                yield
        kop[slot, 64:80, :] = jnp.concatenate(e1_r + e1_i, axis=1).astype(bf)
        kop[slot, 0:64, :] = jnp.concatenate(e2t_r + e2t_i, axis=1).astype(bf)
        yield

    def kgen_mm(d, slot):
        kc = lax.dot_general(kop[slot, 64:80, :], kop[slot, 0:64, :], nt, preferred_element_type=f32)
        xk_s[pl.ds(64 + d, 16, stride=XP), :] = kc

    def u_fwd(a):
        t0 = pl.multiple_of(a * 128, 128)
        aa = lax.dot_general(cst_v[0], uT_s[:, pl.ds(t0, 128)], nt, preferred_element_type=f32)
        for lt in range(4):
            kuh[1, lt, a, 0:128, :] = aa[0:128, 128 * lt:128 * lt + 128]
            kuh[1, lt, a, IMO:IMO + 128, :] = aa[128:256, 128 * lt:128 * lt + 128]

    def k_tr(rho):
        r0 = pl.multiple_of(rho * XP, 4)
        c0 = pl.multiple_of(rho * 64, 64)
        kct_s[pl.ds(c0, 64), :] = xk_s[pl.ds(r0, 512), :].astype(bf).T

    def k_fwd(j):
        g = jnp.where(j < 2, 1, jnp.where(j < 4, 2, jnp.where(j < 8, 3, 4)))
        win = jnp.concatenate(
            [kct_s[pl.ds(pl.multiple_of(tab_s[j * 8 + si], 16), 16), :] for si in range(8)], axis=0)
        kk = jnp.dot(cst_v[g], win, preferred_element_type=f32)
        for lt in range(4):
            kuh[0, lt, j, 0:128, :] = kk[0:128, 128 * lt:128 * lt + 128]
            kuh[0, lt, j, IMO:IMO + 128, :] = kk[128:256, 128 * lt:128 * lt + 128]

    def conv_pair(unit, p, nsplit):
        lt = unit // 16
        r0 = pl.multiple_of((unit % 16) * 8, 8)
        a0 = 2 * p
        a1 = 2 * p + 1
        ar0 = ai0 = ar1 = ai1 = None
        uprev = None
        cuts = set(int(round((a1 + 1) * k / nsplit)) for k in range(1, nsplit))
        for j in range(a1 + 1):
            if j in cuts:
                yield
            kr = kuh[0, lt, j, pl.ds(r0, 8), :]
            ki = kuh[0, lt, j, pl.ds(IMO + r0, 8), :]
            m1 = a1 - j
            if uprev is None:
                u1 = (kuh[1, lt, m1, pl.ds(r0, 8), :], kuh[1, lt, m1, pl.ds(IMO + r0, 8), :])
            else:
                u1 = uprev
            tr = kr * u1[0] - ki * u1[1]
            ti = kr * u1[1] + ki * u1[0]
            ar1 = tr if ar1 is None else ar1 + tr
            ai1 = ti if ai1 is None else ai1 + ti
            m0 = a0 - j
            if m0 >= 0:
                u0 = (kuh[1, lt, m0, pl.ds(r0, 8), :], kuh[1, lt, m0, pl.ds(IMO + r0, 8), :])
                tr = kr * u0[0] - ki * u0[1]
                ti = kr * u0[1] + ki * u0[0]
                ar0 = tr if ar0 is None else ar0 + tr
                ai0 = ti if ai0 is None else ai0 + ti
                uprev = u0
        for a, (yr, yi) in ((a0, (ar0, ai0)), (a1, (ar1, ai1))):
            yf_s[a + 1, lt, pl.ds(r0, 8), :] = yr
            yf_s[a + 1, lt, pl.ds(IMO + r0, 8), :] = yi
        yield

    cim = jnp.concatenate([cst_v[5, 0:128, :], cst_v[5, 128:256, :]], axis=1)
    sgn = jnp.where(lax.broadcasted_iota(jnp.int32, (128, 128), 0) % 2 == 0, np.float32(1.0), np.float32(-1.0))

    def inverse(a):
        t0 = pl.multiple_of(a * 128, 128)
        parts = []
        for lt in range(4):
            yr = yf_s[a + 1, lt, 0:128, :] - sgn * yf_s[a, lt, IMO:IMO + 128, :]
            yi = yf_s[a + 1, lt, IMO:IMO + 128, :] + sgn * yf_s[a, lt, 0:128, :]
            parts.append(jnp.concatenate([yr, yi], axis=0).astype(bf))
        yy = jnp.concatenate(parts, axis=1)
        y = jnp.dot(cim, yy, preferred_element_type=f32).astype(bf)
        st_s[pl.ds(t0, 128), 448:512] = y[:, 64:128]
        st_s[pl.ds(t0, 128), 512:896] = y[:, 128:512]

    NB = NQB * H
    NC = SEQ // CK

    def q_of(i):
        qb = i // H
        h = i % H
        q0 = pl.multiple_of(qb * BQ, BQ)
        return q_s[h, :, pl.ds(q0, BQ)], h

    def pv_chunk(h, c, m, acc):
        s = s_s[pl.ds(c * CK, CK), :]
        p = jnp.exp2(s - m).astype(bf)
        o = jnp.dot(v_s[h, :, pl.ds(c * CK, CK)], p, preferred_element_type=f32)
        return o if acc is None else acc + o

    def p_make(c, m):
        s = s_s[pl.ds(c * CK, CK), :]
        p_s[c % 2, 0:CK, :] = jnp.exp2(s - m).astype(bf)

    def p_make_half(c, m, hf):
        s = s_s[pl.ds(c * CK + hf * (CK // 2), CK // 2), :]
        p_s[c % 2, hf * (CK // 2):(hf + 1) * (CK // 2), :] = jnp.exp2(s - m).astype(bf)

    def pv_mm(h, c, acc):
        o = jnp.dot(v_s[h, :, pl.ds(c * CK, CK)], p_s[c % 2, 0:CK, :], preferred_element_type=f32)
        return o if acc is None else acc + o

    def qk_mm(h, qm, c):
        return jnp.dot(k_s[h, pl.ds(c * CK, CK), 0:32], qm, preferred_element_type=f32)

    def qk_fin(s, c, mrun, pins=None, tasks=()):
        s_s[pl.ds(c * CK, CK), :] = s
        mm = jnp.max(s.reshape(CK // 8, 8, BQ), axis=0)
        if pins is not None:
            groups = pins if isinstance(pins, list) else [pins]
            events = []
            for gi, (pin_store, npin, pinned) in enumerate(groups):
                for k in range(npin):
                    g = (k + 1) * (CK // 8) // npin - 1 if npin > 1 else _OPT.get("pin1_g", 7)
                    if gi > 0:
                        g = (_OPT.get("pk0", 3), _OPT.get("pk1", 11))[k]
                    events.append((g, gi))
            for g, gi in sorted(events):
                pin_store, npin, pinned = groups[gi]
                pin_store(s[8 * g:8 * g + 8, 0:128])
                for t in pinned:
                    next(t, None)
            for pin_store, npin, pinned in groups:
                for t in pinned:
                    for _ in t:
                        pass
        for t in tasks:
            for _ in t:
                pass
        return mm if mrun is None else jnp.maximum(mrun, mm)

    qm0, h0 = q_of(0)
    mrun = None
    for c in range(NC):
        mrun = qk_fin(qk_mm(0, qm0, c), c, mrun)

    cfg = {}

    PSTPIN = _OPT.get('pstpin', [-1, -1])

    def att_step(i, mrun_prev, extra, pst=False, last=False):
        m_cur = jnp.max(mrun_prev, axis=0, keepdims=True)
        inext = jnp.minimum(i + 1, NB - 1)
        qm, hn = q_of(inext)
        qb = i // H
        h = i % H
        mrun = None
        acc = None
        state = {}
        for c in range(NC):
            pre = None
            if extra is not None and _OPT.get("gmode", 0) == 2:
                pre = extra(i, c, state)
                for t in state.pop('pre', []):
                    for _ in t:
                        pass
            if last:
                acc = pv_chunk(h, c, m_cur, acc)
                pins, tasks = (None, ()) if extra is None else extra(i, c, state)
                for t in tasks:
                    for _ in t:
                        pass
                continue
            if pst:
                if c == 0:
                    p_make(0, m_cur)
                acc = pv_mm(h, c, acc)
                s = qk_mm(hn, qm, c)
                if c + 1 < NC:
                    dzp = pl.multiple_of(CK + opaque(i, 13) * 16, 16)
                    for hf in range(2):
                        if PSTPIN[hf] >= 0:
                            g = PSTPIN[hf]
                            p_s[(c + 1) % 2, pl.ds(dzp, 16), 0:128] = jnp.concatenate([s[8 * g:8 * g + 8, 0:128]] * 2, axis=0).astype(bf)
                        p_make_half(c + 1, m_cur, hf)
            elif c < cfg['nqf']:
                s = qk_mm(hn, qm, c)
                acc = pv_chunk(h, c, m_cur, acc)
            else:
                acc = pv_chunk(h, c, m_cur, acc)
                s = qk_mm(hn, qm, c)
            pins, tasks = (None, ()) if extra is None else (pre if pre is not None else extra(i, c, state))
            mrun = qk_fin(s, c, mrun, pins, tasks)
        inv = 1.0 / acc[28:29, :]
        q0 = pl.multiple_of(qb * BQ, BQ)
        o_s[h, :, pl.ds(q0, BQ)] = (acc * inv).astype(bf)
        return mrun


    def run(lo, hi, extra, mrun, name=''):
        pst = name in _OPT.get('pst', [])
        UN = _OPT.get('uns', {}).get(name, 1)
        cfg['nqf'] = _OPT.get('nqfs', {}).get(name, 0)

        def body(t, mrun):
            for u in range(UN):
                mrun = att_step(t * UN + u, mrun, extra, pst)
            return mrun
        return lax.fori_loop(lo // UN, hi // UN, body, mrun)

    def opaque(i, k):
        return (i * k) >> 12

    def fn_task(fn, *a):
        def g():
            fn(*a)
            yield
        return g()

    I_G, I_T, I_KF, I_C, I_I = 4, 32, 36, 40, 56

    def ex_P(i, c, state, fast=False):
        tasks = []
        if c % 4 == 1:
            tasks.append(fn_task(u_fwd, i * 4 + c // 4))
        if _OPT.get("ppin", 1) == 0 or not fast:
            if c in (0, 8):
                r0 = pl.multiple_of(i * 112 + (0 if c == 0 else 48), 16)
                tasks.append(fn_task(bprep, r0, 48 if c == 0 else 64, fast))
            return None, tasks
        gr = _OPT.get("pgr", 16)
        if (gr == 16 and c % 2 == 0 and c < 14) or (gr == 8 and c < 14):
            r0 = pl.multiple_of(i * 112 + 8 * c, 8) if gr == 8 else pl.multiple_of(i * 112 + 16 * (c // 2), 16)
            dzq = pl.multiple_of(D + opaque(i, 9) * 16, 16)

            def pin_store(v):
                dt_s[pl.ds(dzq, 8), :] = v
                par_v[0, pl.ds(dzq, 16), 0:128] = jnp.concatenate([v, v], axis=0).astype(bf)
            return (pin_store, 1, [fn_task(bprep, r0, gr, fast)]), tasks
        return None, tasks

    def ex_G(i, c, state):
        j = i - I_G
        st = c // 8
        dz = pl.multiple_of(448 + opaque(i, 9) * 8, 8)

        def pin_store(v):
            pw[4, pl.ds(dz, 8), 0:128] = v
        tasks = [kgen_chan(2 * j + st, c % 8, st)]
        pinned = []
        if c % 8 == 0:
            nb = 2 * j + 1 if st == 0 else jnp.minimum(2 * j + 2, D // 8 - 1)
            if _OPT.get("ptile", 0):
                state['prep'] = [kgen_prep(nb, 1 - st, (0,)), kgen_prep(nb, 1 - st, (1,))]
            else:
                state['prep'] = [kgen_prep(nb, 1 - st)]
        if c % 8 < 6:
            if _OPT.get("ptile", 0):
                def two(gens=state['prep']):
                    next(gens[0])
                    yield
                    next(gens[1])
                    yield
                pinned.append(two())
            else:
                pinned.append(fn_task(next, state['prep'][0]))
        mode = _OPT.get("gmode", 0)
        if mode == 1:
            dz2 = pl.multiple_of(ONE + opaque(i, 11) * 8, 8)

            def pin_store2(v):
                gss[st][0, pl.ds(dz2, 8), :] = v
            groups = [(pin_store, NPIN_G, pinned)] if pinned else []
            groups.append((pin_store2, 2, tasks))
            return groups, []
        if mode == 3:
            dz2 = pl.multiple_of(ONE + opaque(i, 11) * 8, 8)

            def pin_store2(v):
                gss[st][0, pl.ds(dz2, 8), :] = v
            tasks = []
            if c > 0:
                cp = c - 1
                tasks.append(fn_task(kgen_mm, (2 * j + cp // 8) * 8 + cp % 8, cp % 2))
            gen = kgen_gen(c % 8, st, c % 2)
            if c == NC - 1:
                def last(gen=gen):
                    for _ in gen:
                        pass
                    kgen_mm((2 * j + 1) * 8 + 7, c % 2)
                    yield
                tasks.append(last())
                gen = None
            groups = [(pin_store, NPIN_G, pinned)] if pinned else []
            if gen is not None:
                if _OPT.get("gpin", 1):
                    groups.append((pin_store2, 2, [gen]))
                else:
                    tasks.append(gen)
            return (groups if groups else None), tasks
        if mode == 2:
            state['pre'] = tasks
            tasks = []
        if NPIN_G == 0 or not pinned:
            return None, pinned + tasks
        return (pin_store, 2 if _OPT.get('ptile', 0) else NPIN_G, pinned), tasks

    def ex_T(i, c, state):
        if c % 4 == 1:
            return None, [fn_task(k_tr, (i - I_T) * 4 + c // 4)]
        return None, []

    def ex_KF(i, c, state):
        if c % 4 == 1:
            return None, [fn_task(k_fwd, (i - I_KF) * 4 + c // 4)]
        return None, []

    def ex_C(i, c, state):
        dz = 16 + opaque(i, 9)

        def pin_store(v):
            kuh[0, 0, dz, 0:8, :] = v
        ub = (i - I_C) * 4 + c // 4
        pp = c % 4
        return (pin_store, NPIN_C, [conv_pair(ub, pp, NPIN_C), conv_pair(ub, 7 - pp, NPIN_C)]), []

    def ex_I(i, c, state):
        if c % 8 == 2:
            return None, [fn_task(inverse, (i - I_I) * 2 + c // 8)]
        return None, []

    out_cps = []

    def outproj_body(qb, carry):
        q0 = pl.multiple_of(qb * BQ, BQ)
        oT = o_s[:, :, pl.ds(q0, BQ)].reshape(512, BQ)
        ya = lax.dot_general(oT, wop_s[...], tn, preferred_element_type=f32)
        st_s[pl.ds(q0, BQ), 0:448] = ya.astype(bf)
        pltpu.make_async_copy(st_s.at[pl.ds(q0, BQ), :], out_h.at[0, pl.ds(q0, BQ), :], osem.at[qb]).start()
        return carry

    zmax = jnp.max(jnp.abs(par_v[1, 0:D, :].astype(f32)) * jnp.concatenate([dt_s[0:D, :]] * 2, axis=1))
    mr_s[...] = mrun
    with _scope('P'):
        @pl.when(zmax <= np.float32(8192.0))
        def _():
            mr_s[...] = run(0, I_G, functools.partial(ex_P, fast=True), mr_s[...], 'P')

        @pl.when(jnp.logical_not(zmax <= np.float32(8192.0)))
        def _():
            mr_s[...] = run(0, I_G, ex_P, mr_s[...], 'P')
    mrun = mr_s[...]
    for _ in kgen_prep(0, 0):
        pass
    with _scope('G'):
        mrun = run(I_G, I_T, ex_G, mrun, 'G')
    with _scope('T'):
        mrun = run(I_T, I_KF, ex_T, mrun, 'T')
    with _scope('KF'):
        mrun = run(I_KF, I_C, ex_KF, mrun, 'KF')
    dsk = jnp.concatenate([jnp.zeros((1, 64), f32), dsk_v[...].astype(f32).reshape(1, D)], axis=1)
    for lt in range(4):
        kuh[0, lt, 0, 0:128, :] = kuh[0, lt, 0, 0:128, :] + dsk[:, 128 * lt:128 * lt + 128]
    with _scope('C'):
        mrun = run(I_C, I_I, ex_C, mrun, 'C')
    with _scope('I'):
        if _OPT.get('peel', 1):
            mrun = run(I_I, NB - 1, ex_I, mrun, 'I')
            att_step(NB - 1, mrun, ex_I, last=True)
        else:
            mrun = run(I_I, NB, ex_I, mrun, 'I')
    with _scope('outproj'):
        lax.fori_loop(0, NQB, outproj_body, 0)
    with _scope('outwait'):
      for qb in range(NQB):
        pltpu.make_async_copy(st_s.at[pl.ds(qb * BQ, BQ), :], out_h.at[0, pl.ds(qb * BQ, BQ), :], osem.at[qb]).wait()


@jax.jit
def pallas_concat_heads__mha_block__ssm_conv_s4__prompt_kernel(
        A_x, A_wqkv, A_wo, B_u, B_A_re, B_A_im, B_B_re, B_B_im, B_C_re, B_C_im, B_log_dt, B_Dskip):
    hbm = pl.BlockSpec(memory_space=pltpu.HBM)
    scratch = [
        pltpu.VMEM((D, SEQ), bf),
        pltpu.VMEM((D, 3 * D), bf),
        pltpu.VMEM((D, D), bf),
        pltpu.VMEM((512, SEQ), bf),
        pltpu.VMEM((6, D + 16, NST), bf),
        pltpu.VMEM((D,), bf),
        pltpu.VMEM((D,), bf),
        pltpu.VMEM((6, 256, 128), bf),
        pltpu.VMEM((1352, 128), f32), pltpu.VMEM((1352, 128), f32),
        pltpu.VMEM((1352, 128), f32), pltpu.VMEM((1352, 64), f32),
        pltpu.VMEM((1408, D), bf),
        pltpu.VMEM((D, D), f32),
        pltpu.VMEM((512, D), bf),
        pltpu.VMEM((16, 32, SEQ), bf),
        pltpu.VMEM((16, SEQ, 128), bf),
        pltpu.VMEM((16, 32, SEQ), bf),
        pltpu.VMEM((SEQ, BQ), f32),
        pltpu.VMEM((16, 32, SEQ), bf),
        pltpu.VMEM((5, 456, NST), f32),
        pltpu.VMEM((2, 640, 128), f32), pltpu.VMEM((2, 640, 128), f32),
        pltpu.VMEM((XP * 16, 64), f32),
        pltpu.VMEM((1024, 512), bf),
        pltpu.VMEM((2, 4, 17, PLN, 128), f32),
        pltpu.VMEM((17, 4, PLN, 128), f32),
        pltpu.VMEM((SEQ, 896), bf),
        pltpu.VMEM((D + 16, 128), f32),
        pltpu.VMEM((2, 80, 512), bf),
        pltpu.VMEM((2, CK + 16, BQ), bf),
        pltpu.VMEM((8, BQ), f32),
        pltpu.SMEM((128,), jnp.int32),
        pltpu.SemaphoreType.DMA((21,)),
        pltpu.SemaphoreType.DMA((4,)),
    ]
    c = lambda a: pltpu.with_memory_space_constraint(a, pltpu.HBM)
    xT = jnp.transpose(A_x[0])
    uT = jnp.transpose(B_u[0])
    args = [c(a) for a in (xT, A_wqkv, A_wo, uT, B_A_re, B_A_im, B_B_re, B_B_im, B_C_re, B_C_im,
                           B_log_dt, B_Dskip, jnp.asarray(_CONSTS))]
    return pl.pallas_call(
        _kernel,
        out_shape=jax.ShapeDtypeStruct((1, SEQ, 2 * D), bf),
        in_specs=[hbm] * 13,
        out_specs=hbm,
        scratch_shapes=scratch,
        compiler_params=pltpu.CompilerParams(vmem_limit_bytes=110 * 2 ** 20, flags=_FLAGS),
    )(*args)
```

```python
import functools

import jax
import jax.numpy as jnp
import ml_dtypes
import numpy as np
from jax import lax
from jax.experimental import pallas as pl
from jax.experimental.pallas import tpu as pltpu

bf = jnp.bfloat16
f32 = jnp.float32

SEQ = 2048
D = 448
H = 16
DH = 28
NST = 256
BQ = 512
CK = 128
NQB = SEQ // BQ
NB = NQB * H
NC = SEQ // CK
LOG2E = 1.4426950408889634

XP = 516
IMO = 144
PLN = 280
NPIN_C = 8
PR, PI, ER, EI, MU = 0, 96, 192, 384, 576
I_G, I_T, I_KF, I_C, I_I = 4, 32, 36, 40, 56

_L1 = np.array([0, 1, 2, 3, 4, 5, 6, 7, 512, 516, 1024, 1536, 2048])


def _slabs(j):
    if j < 2:
        return [(r, 16 * j) for r in range(8)]
    if j < 4:
        return [(r, 16 * j) for r in (0, 2, 4, 6)] + [(0, 48) if j == 2 else (8, 0)]
    if j < 8:
        return [(8, 16 * (j - 4)), (9, 16 * (j - 4))] + [(8, 16 * (j - 3)) if j < 7 else (10, 0)]
    if j < 12:
        return [(10, 16 * (j - 8))] + [(10, 16 * (j - 7)) if j < 11 else (11, 0)]
    return [(11, 16 * (j - 12))] + [(11, 16 * (j - 11)) if j < 15 else (12, 0)]


def _slab_rows(j):
    rows = [64 * rho + c0 for rho, c0 in _slabs(j)]
    return rows + [rows[0]] * (8 - len(rows))


def _make_consts():
    k = np.arange(128)[:, None]
    n = np.arange(128)[None, :]
    ang = np.pi * (2 * k + 1) * n / 256.0
    ct = np.concatenate([np.cos(ang), -np.sin(ang)], 0)
    ci = np.concatenate([np.cos(ang.T), -np.sin(ang.T)], 1) / 128.0
    out = np.zeros((6, 256, 128), np.float64)
    out[0] = ct
    for g, j in enumerate((0, 2, 4, 8)):
        pos = {}
        for si, (rho, c0) in enumerate(_slabs(j)):
            for cc in range(16):
                pos.setdefault(int(_L1[rho] + 8 * (c0 + cc)), si * 16 + cc)
        for nn in range(128):
            lag = int(np.float32(128 * j + nn).astype(ml_dtypes.bfloat16).astype(np.float32))
            out[g + 1][:, pos[lag]] += ct[:, nn]
    out[5, 0:128] = ci[:, 0:128]
    out[5, 128:256] = ci[:, 128:256]
    return out.astype(np.float32).astype(ml_dtypes.bfloat16)


_CONSTS = _make_consts()


def _cmul(ar, ai, br, bi):
    return ar * br - ai * bi, ar * bi + ai * br


def _cmulc(ar, ai, br, bi):
    return ar * br + ai * bi, ai * br - ar * bi


def _csq(ar, ai):
    return ar * ar - ai * ai, (ar + ar) * ai


def _sincos(x):
    kf = jnp.round(x * np.float32(2.0 / np.pi))
    ki = kf.astype(jnp.int32)
    r = x - kf * np.float32(1.5703125)
    r = r - kf * np.float32(4.837512969970703125e-4)
    r = r - kf * np.float32(7.54978995489188216e-8)
    r2 = r * r
    s = r + r * r2 * (np.float32(-1.6666654611e-1)
                      + r2 * (np.float32(8.3321608736e-3) + r2 * np.float32(-1.9515295891e-4)))
    c = (np.float32(1.0) - np.float32(0.5) * r2) + r2 * r2 * (
        np.float32(4.166664568298827e-2)
        + r2 * (np.float32(-1.388731625493765e-3) + r2 * np.float32(2.443315711809948e-5)))
    swap = (ki & 1) == 1
    sb = jnp.where(swap, c, s)
    cb = jnp.where(swap, s, c)
    return jnp.where((ki & 2) != 0, -sb, sb), jnp.where(((ki + 1) & 2) != 0, -cb, cb)


def _task(fn, *args):
    def g():
        fn(*args)
        yield
    return g()


def _drain(tasks):
    for t in tasks:
        for _ in t:
            pass


def _opaque0(i, k):
    return (i * k) >> 12


_NT = (((1,), (1,)), ((), ()))
_TN = (((0,), (0,)), ((), ()))


def _kernel(xT_h, wqkv_h, wo_h, uT_h, are_h, aim_h, bre_h, bim_h, cre_h, cim_h, ldt_h, dsk_h, cst_h,
            out_h,
            xT_v, wqkv_v, wo_v, uT_s, par_v, ldt_v, dsk_v, cst_v,
            wt0, wt1, wt2, wt3, wp_s, wo_f, wop_s,
            q_s, k_s, v_s, s_s, o_s,
            pw, gs0, gs1, xk_s, kct_s, kuh, yf_s, st_s, dt_s, mr_s, tab_s, sems, osem):
    gss = (gs0, gs1)
    wts = (wt0, wt1, wt2, wt3)

    cp_w = [pltpu.make_async_copy(wqkv_h.at[pl.ds(128 * t, 64 if t == 3 else 128), :],
                                  wqkv_v.at[pl.ds(128 * t, 64 if t == 3 else 128), :], sems.at[17 + t])
            for t in range(4)]

    def x_copy(b):
        t0 = pl.multiple_of(b * 512, 512)
        return pltpu.make_async_copy(xT_h.at[:, pl.ds(t0, 512)], xT_v.at[:, pl.ds(t0, 512)], sems.at[13 + b])
    cp_par = [pltpu.make_async_copy(r, par_v.at[i, pl.ds(0, D), :], sems.at[2 + i])
              for i, r in enumerate((are_h, aim_h, bre_h, bim_h, cre_h, cim_h))]
    cp_ldt = pltpu.make_async_copy(ldt_h, ldt_v, sems.at[8])
    cp_dsk = pltpu.make_async_copy(dsk_h, dsk_v, sems.at[9])
    cp_cst = pltpu.make_async_copy(cst_h, cst_v, sems.at[10])
    cp_wo = pltpu.make_async_copy(wo_h, wo_v, sems.at[11])
    cp_u = pltpu.make_async_copy(uT_h, uT_s.at[pl.ds(64, D), :], sems.at[12])
    for c in cp_w:
        c.start()
    x_copy(0).start()
    x_copy(1).start()
    for c in cp_par:
        c.start()
    cp_ldt.start()
    x_copy(2).start()
    x_copy(3).start()
    cp_dsk.start()
    cp_cst.start()
    cp_wo.start()
    cp_u.start()

    uT_s[0:64, :] = jnp.zeros((64, SEQ), bf)
    for j in range(16):
        for si, r in enumerate(_slab_rows(j)):
            tab_s[j * 8 + si] = np.int32(r)
    for gs in gss:
        for t in range(2):
            gs[t, ER + 13 * 12:ER + 16 * 12, :] = jnp.zeros((36, 128), f32)
            gs[t, EI + 13 * 12:EI + 16 * 12, :] = jnp.zeros((36, 128), f32)
    for rho in range(16):
        xk_s[XP * rho:XP * rho + 64, :] = jnp.zeros((64, 64), f32)
    for lt in range(4):
        yf_s[0, lt, 0:128, :] = jnp.zeros((128, 128), f32)
        yf_s[0, lt, IMO:IMO + 128, :] = jnp.zeros((128, 128), f32)

    for t in range(4):
        w = 64 if t == 3 else 128
        cols = slice(128 * t, 128 * t + w)
        cp_w[t].wait()
        wT = wqkv_v[cols, :].T.astype(f32)
        wts[t][0:1344, :] = wT
        wts[t][1344:1352, :] = jnp.zeros((8, w), f32)
        wp_s[0:448, cols] = wT[0:448].astype(bf)
        wp_s[960:1408, cols] = wT[896:1344].astype(bf)
        for hh in range(H):
            wp_s[448 + 32 * hh:448 + 32 * hh + 32, cols] = wts[t][pl.ds(448 + 28 * hh, 32), :].astype(bf)

    zpad = jnp.zeros((4, 512), f32)
    opad = jnp.where(lax.broadcasted_iota(jnp.int32, (4, 512), 0) == 0, np.float32(1.0), np.float32(0.0))

    def proj_body(b, carry):
        t0 = pl.multiple_of(b * 512, 512)
        x_copy(b).wait()
        xb = xT_v[:, pl.ds(t0, 512)]
        kT = jnp.dot(wp_s[448:960, :], xb, preferred_element_type=f32)
        qq = jnp.dot(wp_s[0:448, :], xb, preferred_element_type=f32) * np.float32(DH ** -0.5 * LOG2E)
        for hh in range(H):
            q_s[hh, :, pl.ds(t0, 512)] = jnp.concatenate([qq[28 * hh:28 * hh + 28, :], zpad], axis=0).astype(bf)
        vv = jnp.dot(wp_s[960:1408, :], xb, preferred_element_type=f32)
        for hh in range(H):
            v_s[hh, :, pl.ds(t0, 512)] = jnp.concatenate([vv[28 * hh:28 * hh + 28, :], opad], axis=0).astype(bf)
        for g in range(4):
            kg = kT[128 * g:128 * g + 128, :].T
            k_s[4 * g, pl.ds(t0, 512), :] = kg.astype(bf)
            for j in range(1, 4):
                k_s[4 * g + j, pl.ds(t0, 512), :] = pltpu.roll(kg, 128 - 32 * j, 1).astype(bf)
        return carry
    lax.fori_loop(0, 4, proj_body, 0)

    for c in cp_par:
        c.wait()
    cp_ldt.wait()
    dt_row = jnp.exp(ldt_v[...].astype(f32).reshape(1, D)).astype(bf).astype(f32)
    dt_s[0:D, :] = jnp.broadcast_to(dt_row, (128, D)).T
    cp_cst.wait()
    cp_u.wait()
    cp_dsk.wait()
    cp_wo.wait()
    wo_f[...] = wo_v[...].astype(f32)
    for hh in range(H):
        wop_s[32 * hh:32 * hh + 32, :] = jnp.concatenate(
            [wo_f[28 * hh:28 * hh + 28, :], jnp.zeros((4, D), f32)], axis=0).astype(bf)

    def bprep(r0, n, fast):
        sl = pl.ds(r0, n)
        dtc = dt_s[sl, :]
        dt2 = jnp.concatenate([dtc, dtc], axis=1)
        zr = dt2 * par_v[0, sl, :].astype(f32)
        zi = dt2 * par_v[1, sl, :].astype(f32)
        dbr = dt2 * par_v[2, sl, :].astype(f32)
        dbi = dt2 * par_v[3, sl, :].astype(f32)
        wr, wi = _cmul(par_v[4, sl, :].astype(f32), par_v[5, sl, :].astype(f32), dbr, dbi)
        pw[2, sl, :] = wr
        pw[3, sl, :] = wi
        mag = jnp.exp(zr)
        sn, cs = _sincos(zi) if fast else (jnp.sin(zi), jnp.cos(zi))
        pw[0, sl, :] = mag * cs
        pw[1, sl, :] = mag * sn

    def kgen_prep(b, st):
        d0 = pl.multiple_of(b * 8, 8)
        gs = gss[st]

        def ld(k):
            return pw[k, pl.ds(d0, 8), :], pw[k + 1, pl.ds(d0, 8), :]

        def tmp_ld(k):
            r = 48 * st + 16 * k
            return pw[4, r:r + 8, :], pw[4, r + 8:r + 16, :]

        def tmp_st(k, v):
            r = 48 * st + 16 * k
            pw[4, r:r + 8, :] = v[0]
            pw[4, r + 8:r + 16, :] = v[1]

        def put_rows(rr, ri, val):
            for t in range(2):
                gs[t, rr:rr + 8, :] = val[0][:, 128 * t:128 * t + 128]
                gs[t, ri:ri + 8, :] = val[1][:, 128 * t:128 * t + 128]

        def get_rows(rr, ri):
            return tuple(jnp.concatenate([gs[t, r:r + 8, :] for t in range(2)], axis=1) for r in (rr, ri))

        def put_e(idx, val):
            put_rows(ER + 12 * idx, EI + 12 * idx, val)

        def put_p(idx, val):
            put_rows(PR + 12 * idx, PI + 12 * idx, val)

        def get_p(idx):
            return get_rows(PR + 12 * idx, PI + 12 * idx)

        e1, w = ld(0), ld(2)
        put_e(0, w)
        put_e(1, _cmul(*w, *e1))
        e2 = _csq(*e1)
        put_e(2, _cmul(*w, *e2))
        tmp_st(0, e2)
        tmp_st(1, _cmul(*e2, *e1))
        yield
        w, e2, e3 = ld(2), tmp_ld(0), tmp_ld(1)
        put_e(3, _cmul(*w, *e3))
        e4 = _csq(*e2)
        tmp_st(2, e4)
        put_e(4, _cmul(*w, *e4))
        put_e(6, _cmul(*w, *_csq(*e3)))
        yield
        e1, w, e3, e4 = ld(0), ld(2), tmp_ld(1), tmp_ld(2)
        put_e(5, _cmul(*w, *_cmul(*e4, *e1)))
        put_e(7, _cmul(*w, *_cmul(*e4, *e3)))
        e8 = _csq(*e4)
        put_p(0, (jnp.ones_like(e8[0]), jnp.zeros_like(e8[0])))
        put_p(1, (e8[0], -e8[1]))
        yield
        p1 = get_p(1)
        p2 = _csq(*p1)
        put_p(2, p2)
        p3 = _cmul(*p2, *p1)
        put_p(3, p3)
        p4 = _csq(*p2)
        put_p(4, p4)
        put_p(5, _cmul(*p4, *p1))
        put_p(6, _csq(*p3))
        yield
        p3, p4 = get_p(3), get_p(4)
        put_p(7, _cmul(*p4, *p3))
        m8 = _csq(*p4)
        put_rows(MU, MU + 8, m8)
        m16 = _csq(*m8)
        put_rows(MU + 16, MU + 24, m16)
        put_rows(MU + 32, MU + 40, _csq(*m16))
        yield
        w, e4, m32 = ld(2), tmp_ld(2), get_rows(MU + 32, MU + 40)
        x512 = _csq(*m32)
        w512 = _cmulc(*w, *x512)
        put_e(8, w512)
        put_e(9, _cmul(*w512, *e4))
        x1024 = _csq(*x512)
        put_e(10, _cmulc(*w, *x1024))
        put_e(11, _cmulc(*w, *_cmul(*x1024, *x512)))
        put_e(12, _cmulc(*w, *_csq(*x1024)))
        yield

    def kgen_chan(b, i, st):
        gs = gss[st]
        e2_r, e2_i, e1_r, e1_i = [], [], [], []
        for t in range(2):
            b0 = (gs[t, pl.ds(PR + i, 8, stride=12), :], gs[t, pl.ds(PI + i, 8, stride=12), :])
            m8, m16, m32 = [(jnp.broadcast_to(gs[t, pl.ds(MU + 16 * k + i, 1), :], (8, 128)),
                             jnp.broadcast_to(gs[t, pl.ds(MU + 16 * k + 8 + i, 1), :], (8, 128)))
                            for k in range(3)]
            b1 = _cmul(*b0, *m8)
            b2 = _cmul(*b0, *m16)
            b3 = _cmul(*b1, *m16)
            blks = (b0, b1, b2, b3, _cmul(*b0, *m32), _cmul(*b1, *m32), _cmul(*b2, *m32), _cmul(*b3, *m32))
            e2_r.append(jnp.concatenate([v[0] for v in blks], axis=0))
            e2_i.append(jnp.concatenate([v[1] for v in blks], axis=0))
            e1_r.append(gs[t, pl.ds(ER + i, 16, stride=12), :])
            e1_i.append(gs[t, pl.ds(EI + i, 16, stride=12), :])
        lhs = jnp.concatenate(e1_r + e1_i, axis=1).astype(bf)
        rhs = jnp.concatenate(e2_r + e2_i, axis=1).astype(bf)
        kc = lax.dot_general(lhs, rhs, _NT, preferred_element_type=f32)
        xk_s[pl.ds(64 + b * 8 + i, 16, stride=XP), :] = kc

    def put_spectrum(which, idx, val):
        for lt in range(4):
            kuh[which, lt, idx, 0:128, :] = val[0:128, 128 * lt:128 * lt + 128]
            kuh[which, lt, idx, IMO:IMO + 128, :] = val[128:256, 128 * lt:128 * lt + 128]

    def u_fwd(a):
        t0 = pl.multiple_of(a * 128, 128)
        put_spectrum(1, a, lax.dot_general(cst_v[0], uT_s[:, pl.ds(t0, 128)], _NT, preferred_element_type=f32))

    def k_tr(rho):
        r0 = pl.multiple_of(rho * XP, 4)
        c0 = pl.multiple_of(rho * 64, 64)
        kct_s[pl.ds(c0, 64), :] = xk_s[pl.ds(r0, 512), :].astype(bf).T

    def k_fwd(j):
        g = jnp.where(j < 2, 1, jnp.where(j < 4, 2, jnp.where(j < 8, 3, 4)))
        win = jnp.concatenate(
            [kct_s[pl.ds(pl.multiple_of(tab_s[j * 8 + si], 16), 16), :] for si in range(8)], axis=0)
        put_spectrum(0, j, jnp.dot(cst_v[g], win, preferred_element_type=f32))

    def conv_pair(unit, p):
        lt = unit // 16
        r0 = pl.multiple_of((unit % 16) * 8, 8)

        def ld(which, idx):
            return kuh[which, lt, idx, pl.ds(r0, 8), :], kuh[which, lt, idx, pl.ds(IMO + r0, 8), :]

        def mac(acc, k, u):
            t = (k[0] * u[0] - k[1] * u[1], k[0] * u[1] + k[1] * u[0])
            return t if acc is None else (acc[0] + t[0], acc[1] + t[1])
        a0, a1 = 2 * p, 2 * p + 1
        y0 = y1 = uprev = None
        cuts = set(int(round((a1 + 1) * k / NPIN_C)) for k in range(1, NPIN_C))
        for j in range(a1 + 1):
            if j in cuts:
                yield
            k = ld(0, j)
            y1 = mac(y1, k, ld(1, a1 - j) if uprev is None else uprev)
            if a0 - j >= 0:
                uprev = ld(1, a0 - j)
                y0 = mac(y0, k, uprev)
        for a, y in ((a0, y0), (a1, y1)):
            yf_s[a + 1, lt, pl.ds(r0, 8), :] = y[0]
            yf_s[a + 1, lt, pl.ds(IMO + r0, 8), :] = y[1]
        yield

    cinv = jnp.concatenate([cst_v[5, 0:128, :], cst_v[5, 128:256, :]], axis=1)
    sgn = jnp.where(lax.broadcasted_iota(jnp.int32, (128, 128), 0) % 2 == 0, np.float32(1.0), np.float32(-1.0))

    def inverse(a):
        t0 = pl.multiple_of(a * 128, 128)
        parts = []
        for lt in range(4):
            yr = yf_s[a + 1, lt, 0:128, :] - sgn * yf_s[a, lt, IMO:IMO + 128, :]
            yi = yf_s[a + 1, lt, IMO:IMO + 128, :] + sgn * yf_s[a, lt, 0:128, :]
            parts.append(jnp.concatenate([yr, yi], axis=0).astype(bf))
        y = jnp.dot(cinv, jnp.concatenate(parts, axis=1), preferred_element_type=f32).astype(bf)
        st_s[pl.ds(t0, 128), 448:512] = y[:, 64:128]
        st_s[pl.ds(t0, 128), 512:896] = y[:, 128:512]

    def ex_P(i, c, state, fast):
        tasks = [_task(u_fwd, i * 4 + c // 4)] if c % 4 == 1 else []
        if not fast:
            if c in (0, 8):
                r0 = pl.multiple_of(i * 112 + (0 if c == 0 else 48), 16)
                tasks.append(_task(bprep, r0, 48 if c == 0 else 64, False))
            return None, tasks
        if c >= 14:
            return None, tasks
        spare = pl.multiple_of(D + _opaque0(i, 9) * 16, 16)

        def pin(v):
            dt_s[pl.ds(spare, 8), :] = v
            par_v[0, pl.ds(spare, 16), 0:128] = jnp.concatenate([v, v], axis=0).astype(bf)
        return (pin, 1, [_task(bprep, pl.multiple_of(i * 112 + 8 * c, 8), 8, True)]), tasks

    def ex_G(i, c, state):
        j = i - I_G
        st = c // 8
        spare = pl.multiple_of(D + _opaque0(i, 9) * 8, 8)

        def pin(v):
            pw[4, pl.ds(spare, 8), 0:128] = v
        tasks = [_task(kgen_chan, 2 * j + st, c % 8, st)]
        if c % 8 == 0:
            state['prep'] = kgen_prep(2 * j + 1 if st == 0 else jnp.minimum(2 * j + 2, D // 8 - 1), 1 - st)
        if c % 8 < 6:
            return (pin, 1, [_task(next, state['prep'])]), tasks
        return None, tasks

    def ex_T(i, c, state):
        return None, ([_task(k_tr, (i - I_T) * 4 + c // 4)] if c % 4 == 1 else [])

    def ex_KF(i, c, state):
        return None, ([_task(k_fwd, (i - I_KF) * 4 + c // 4)] if c % 4 == 1 else [])

    def ex_C(i, c, state):
        spare = 16 + _opaque0(i, 9)

        def pin(v):
            kuh[0, 0, spare, 0:8, :] = v
        unit = (i - I_C) * 4 + c // 4
        return (pin, NPIN_C, [conv_pair(unit, c % 4), conv_pair(unit, 7 - c % 4)]), []

    def ex_I(i, c, state):
        return None, ([_task(inverse, (i - I_I) * 2 + c // 8)] if c % 8 == 2 else [])

    def q_of(i):
        return q_s[i % H, :, pl.ds(pl.multiple_of((i // H) * BQ, BQ), BQ)], i % H

    def pv_chunk(h, c, m, acc):
        p = jnp.exp2(s_s[pl.ds(c * CK, CK), :] - m).astype(bf)
        o = jnp.dot(v_s[h, :, pl.ds(c * CK, CK)], p, preferred_element_type=f32)
        return o if acc is None else acc + o

    def qk_chunk(h, q, c):
        return jnp.dot(k_s[h, pl.ds(c * CK, CK), 0:32], q, preferred_element_type=f32)

    def qk_keep(s, c, mrun, pins=None, tasks=()):
        s_s[pl.ds(c * CK, CK), :] = s
        mm = jnp.max(s.reshape(CK // 8, 8, BQ), axis=0)
        if pins is not None:
            pin, npin, pinned = pins
            for k in range(npin):
                g = (k + 1) * (CK // 8) // npin - 1
                pin(s[8 * g:8 * g + 8, 0:128])
                for t in pinned:
                    next(t, None)
            _drain(pinned)
        _drain(tasks)
        return mm if mrun is None else jnp.maximum(mrun, mm)

    def att_step(i, mrun_prev, extra, nqf, last=False):
        m = jnp.max(mrun_prev, axis=0, keepdims=True)
        if not last:
            qn, hn = q_of(jnp.minimum(i + 1, NB - 1))
        h = i % H
        mrun = acc = None
        state = {}
        for c in range(NC):
            if last:
                acc = pv_chunk(h, c, m, acc)
                _drain(extra(i, c, state)[1])
                continue
            if c < nqf:
                s = qk_chunk(hn, qn, c)
                acc = pv_chunk(h, c, m, acc)
            else:
                acc = pv_chunk(h, c, m, acc)
                s = qk_chunk(hn, qn, c)
            mrun = qk_keep(s, c, mrun, *extra(i, c, state))
        inv = 1.0 / acc[28:29, :]
        o_s[h, :, pl.ds(pl.multiple_of((i // H) * BQ, BQ), BQ)] = (acc * inv).astype(bf)
        return mrun

    def run(lo, hi, extra, mrun, nqf, unroll=1):
        def body(t, mrun):
            for u in range(unroll):
                mrun = att_step(t * unroll + u, mrun, extra, nqf)
            return mrun
        return lax.fori_loop(lo // unroll, hi // unroll, body, mrun)

    q0, _ = q_of(0)
    mrun = None
    for c in range(NC):
        mrun = qk_keep(qk_chunk(0, q0, c), c, mrun)

    zmax = jnp.max(jnp.abs(par_v[1, 0:D, :].astype(f32)) * jnp.concatenate([dt_s[0:D, :]] * 2, axis=1))
    mr_s[...] = mrun

    @pl.when(zmax <= np.float32(8192.0))
    def _():
        mr_s[...] = run(0, I_G, functools.partial(ex_P, fast=True), mr_s[...], 0)

    @pl.when(jnp.logical_not(zmax <= np.float32(8192.0)))
    def _():
        mr_s[...] = run(0, I_G, functools.partial(ex_P, fast=False), mr_s[...], 0)

    mrun = mr_s[...]
    _drain([kgen_prep(0, 0)])
    mrun = run(I_G, I_T, ex_G, mrun, 3, unroll=2)
    mrun = run(I_T, I_KF, ex_T, mrun, 2)
    mrun = run(I_KF, I_C, ex_KF, mrun, 2)
    dsk = jnp.concatenate([jnp.zeros((1, 64), f32), dsk_v[...].astype(f32).reshape(1, D)], axis=1)
    for lt in range(4):
        kuh[0, lt, 0, 0:128, :] = kuh[0, lt, 0, 0:128, :] + dsk[:, 128 * lt:128 * lt + 128]
    mrun = run(I_C, I_I, ex_C, mrun, 16, unroll=2)
    mrun = run(I_I, NB - 1, ex_I, mrun, 2)
    att_step(NB - 1, mrun, ex_I, 0, last=True)

    def out_copy(qb):
        q0 = pl.multiple_of(qb * BQ, BQ)
        return pltpu.make_async_copy(st_s.at[pl.ds(q0, BQ), :], out_h.at[0, pl.ds(q0, BQ), :], osem.at[qb])

    def outproj_body(qb, carry):
        q0 = pl.multiple_of(qb * BQ, BQ)
        oT = o_s[:, :, pl.ds(q0, BQ)].reshape(512, BQ)
        ya = lax.dot_general(oT, wop_s[...], _TN, preferred_element_type=f32)
        st_s[pl.ds(q0, BQ), 0:448] = ya.astype(bf)
        out_copy(qb).start()
        return carry
    lax.fori_loop(0, NQB, outproj_body, 0)
    for qb in range(NQB):
        out_copy(qb).wait()


@jax.jit
def pallas_concat_heads__mha_block__ssm_conv_s4__prompt_kernel(
    A_x: jax.Array,
    A_wqkv: jax.Array,
    A_wo: jax.Array,
    B_u: jax.Array,
    B_A_re: jax.Array,
    B_A_im: jax.Array,
    B_B_re: jax.Array,
    B_B_im: jax.Array,
    B_C_re: jax.Array,
    B_C_im: jax.Array,
    B_log_dt: jax.Array,
    B_Dskip: jax.Array,
):
    scratch = [
        pltpu.VMEM((D, SEQ), bf),
        pltpu.VMEM((D, 3 * D), bf),
        pltpu.VMEM((D, D), bf),
        pltpu.VMEM((512, SEQ), bf),
        pltpu.VMEM((6, D + 16, NST), bf),
        pltpu.VMEM((D,), bf),
        pltpu.VMEM((D,), bf),
        pltpu.VMEM((6, 256, 128), bf),
        pltpu.VMEM((1352, 128), f32),
        pltpu.VMEM((1352, 128), f32),
        pltpu.VMEM((1352, 128), f32),
        pltpu.VMEM((1352, 64), f32),
        pltpu.VMEM((1408, D), bf),
        pltpu.VMEM((D, D), f32),
        pltpu.VMEM((512, D), bf),
        pltpu.VMEM((H, 32, SEQ), bf),
        pltpu.VMEM((H, SEQ, 128), bf),
        pltpu.VMEM((H, 32, SEQ), bf),
        pltpu.VMEM((SEQ, BQ), f32),
        pltpu.VMEM((H, 32, SEQ), bf),
        pltpu.VMEM((5, D + 8, NST), f32),
        pltpu.VMEM((2, 640, 128), f32),
        pltpu.VMEM((2, 640, 128), f32),
        pltpu.VMEM((XP * 16, 64), f32),
        pltpu.VMEM((1024, 512), bf),
        pltpu.VMEM((2, 4, 17, PLN, 128), f32),
        pltpu.VMEM((17, 4, PLN, 128), f32),
        pltpu.VMEM((SEQ, 2 * D), bf),
        pltpu.VMEM((D + 16, 128), f32),
        pltpu.VMEM((8, BQ), f32),
        pltpu.SMEM((128,), jnp.int32),
        pltpu.SemaphoreType.DMA((21,)),
        pltpu.SemaphoreType.DMA((NQB,)),
    ]
    hbm = pl.BlockSpec(memory_space=pltpu.HBM)
    operands = (jnp.transpose(A_x[0]), A_wqkv, A_wo, jnp.transpose(B_u[0]), B_A_re, B_A_im, B_B_re, B_B_im,
                B_C_re, B_C_im, B_log_dt, B_Dskip, jnp.asarray(_CONSTS))
    return pl.pallas_call(
        _kernel,
        out_shape=jax.ShapeDtypeStruct((1, SEQ, 2 * D), bf),
        in_specs=[hbm] * len(operands),
        out_specs=hbm,
        scratch_shapes=scratch,
        compiler_params=pltpu.CompilerParams(vmem_limit_bytes=110 * 2 ** 20),
    )(*[pltpu.with_memory_space_constraint(a, pltpu.HBM) for a in operands])
```

```python
import functools

import jax
import jax.numpy as jnp
import ml_dtypes
import numpy as np
from jax import lax
from jax.experimental import pallas as pl
from jax.experimental.pallas import tpu as pltpu

bf = jnp.bfloat16
f32 = jnp.float32

SEQ = 2048
D = 448
H = 16
DH = 28
NST = 256
BQ = 512
CK = 128
NQB = SEQ // BQ
NB = NQB * H
NC = SEQ // CK
LOG2E = 1.4426950408889634

XP = 516
IMO = 144
PLN = 280
OPC = 7
NPIN_C = 8
PR, PI, ER, EI, MU = 0, 96, 192, 384, 576
I_G, I_T, I_KF, I_C, I_I = 4, 32, 36, 40, 56

_L1 = np.array([0, 1, 2, 3, 4, 5, 6, 7, 512, 516, 1024, 1536, 2048])


def _slabs(j):
    if j < 2:
        return [(r, 16 * j) for r in range(8)]
    if j < 4:
        return [(r, 16 * j) for r in (0, 2, 4, 6)] + [(0, 48) if j == 2 else (8, 0)]
    if j < 8:
        return [(8, 16 * (j - 4)), (9, 16 * (j - 4))] + [(8, 16 * (j - 3)) if j < 7 else (10, 0)]
    if j < 12:
        return [(10, 16 * (j - 8))] + [(10, 16 * (j - 7)) if j < 11 else (11, 0)]
    return [(11, 16 * (j - 12))] + [(11, 16 * (j - 11)) if j < 15 else (12, 0)]


def _slab_rows(j):
    rows = [64 * rho + c0 for rho, c0 in _slabs(j)]
    return rows + [rows[0]] * (8 - len(rows))


def _make_consts():
    k = np.arange(128)[:, None]
    n = np.arange(128)[None, :]
    ang = np.pi * (2 * k + 1) * n / 256.0
    ct = np.concatenate([np.cos(ang), -np.sin(ang)], 0)
    ci = np.concatenate([np.cos(ang.T), -np.sin(ang.T)], 1) / 128.0
    out = np.zeros((6, 256, 128), np.float64)
    out[0] = ct
    for g, j in enumerate((0, 2, 4, 8)):
        pos = {}
        for si, (rho, c0) in enumerate(_slabs(j)):
            for cc in range(16):
                pos.setdefault(int(_L1[rho] + 8 * (c0 + cc)), si * 16 + cc)
        for nn in range(128):
            lag = int(np.float32(128 * j + nn).astype(ml_dtypes.bfloat16).astype(np.float32))
            out[g + 1][:, pos[lag]] += ct[:, nn]
    out[5, 0:128] = ci[:, 0:128]
    out[5, 128:256] = ci[:, 128:256]
    return out.astype(np.float32).astype(ml_dtypes.bfloat16)


_CONSTS = _make_consts()


def _cmul(ar, ai, br, bi):
    return ar * br - ai * bi, ar * bi + ai * br


def _cmulc(ar, ai, br, bi):
    return ar * br + ai * bi, ai * br - ar * bi


def _csq(ar, ai):
    return ar * ar - ai * ai, (ar + ar) * ai


def _sincos(x):
    kf = jnp.round(x * np.float32(2.0 / np.pi))
    ki = kf.astype(jnp.int32)
    r = x - kf * np.float32(1.5703125)
    r = r - kf * np.float32(4.837512969970703125e-4)
    r = r - kf * np.float32(7.54978995489188216e-8)
    r2 = r * r
    s = r + r * r2 * (np.float32(-1.6666654611e-1)
                      + r2 * (np.float32(8.3321608736e-3) + r2 * np.float32(-1.9515295891e-4)))
    c = (np.float32(1.0) - np.float32(0.5) * r2) + r2 * r2 * (
        np.float32(4.166664568298827e-2)
        + r2 * (np.float32(-1.388731625493765e-3) + r2 * np.float32(2.443315711809948e-5)))
    swap = (ki & 1) == 1
    sb = jnp.where(swap, c, s)
    cb = jnp.where(swap, s, c)
    return jnp.where((ki & 2) != 0, -sb, sb), jnp.where(((ki + 1) & 2) != 0, -cb, cb)


def _task(fn, *args):
    def g():
        fn(*args)
        yield
    return g()


def _drain(tasks):
    for t in tasks:
        for _ in t:
            pass


def _opaque0(i, k):
    return (i * k) >> 12


_NT = (((1,), (1,)), ((), ()))
_TN = (((0,), (0,)), ((), ()))


def _kernel(xT_h, wqkv_h, wo_h, uT_h, are_h, aim_h, bre_h, bim_h, cre_h, cim_h, ldt_h, dsk_h, cst_h,
            out_h,
            xT_v, wqkv_v, wo_v, uT_s, par_v, ldt_v, dsk_v, cst_v,
            wt0, wt1, wt2, wt3, wp_s, wo_f, wop_s,
            q_s, k_s, v_s, s_s, o_s,
            pw, gs0, gs1, xk_s, kct_s, kuh, yf_s, st_s, dt_s, mr_s, tab_s, sems, osem):
    gss = (gs0, gs1)
    wts = (wt0, wt1, wt2, wt3)

    cp_w = [pltpu.make_async_copy(wqkv_h.at[pl.ds(128 * t, 64 if t == 3 else 128), :],
                                  wqkv_v.at[pl.ds(128 * t, 64 if t == 3 else 128), :], sems.at[17 + t])
            for t in range(4)]

    def x_copy(b):
        t0 = pl.multiple_of(b * 512, 512)
        return pltpu.make_async_copy(xT_h.at[:, pl.ds(t0, 512)], xT_v.at[:, pl.ds(t0, 512)], sems.at[13 + b])
    cp_par = [pltpu.make_async_copy(r, par_v.at[i, pl.ds(0, D), :], sems.at[2 + i])
              for i, r in enumerate((are_h, aim_h, bre_h, bim_h, cre_h, cim_h))]
    cp_ldt = pltpu.make_async_copy(ldt_h, ldt_v, sems.at[8])
    cp_dsk = pltpu.make_async_copy(dsk_h, dsk_v, sems.at[9])
    cp_cst = pltpu.make_async_copy(cst_h, cst_v, sems.at[10])
    cp_wo = pltpu.make_async_copy(wo_h, wo_v, sems.at[11])
    cp_u = pltpu.make_async_copy(uT_h, uT_s.at[pl.ds(64, D), :], sems.at[12])
    for c in cp_w:
        c.start()
    x_copy(0).start()
    x_copy(1).start()
    for c in cp_par:
        c.start()
    cp_ldt.start()
    x_copy(2).start()
    x_copy(3).start()
    cp_dsk.start()
    cp_cst.start()
    cp_wo.start()
    cp_u.start()

    uT_s[0:64, :] = jnp.zeros((64, SEQ), bf)
    for j in range(16):
        for si, r in enumerate(_slab_rows(j)):
            tab_s[j * 8 + si] = np.int32(r)
    for gs in gss:
        for t in range(2):
            gs[t, ER + 13 * 12:ER + 16 * 12, :] = jnp.zeros((36, 128), f32)
            gs[t, EI + 13 * 12:EI + 16 * 12, :] = jnp.zeros((36, 128), f32)
    for rho in range(16):
        xk_s[XP * rho:XP * rho + 64, :] = jnp.zeros((64, 64), f32)
    for lt in range(4):
        yf_s[0, lt, 0:128, :] = jnp.zeros((128, 128), f32)
        yf_s[0, lt, IMO:IMO + 128, :] = jnp.zeros((128, 128), f32)

    for t in range(4):
        w = 64 if t == 3 else 128
        cols = slice(128 * t, 128 * t + w)
        cp_w[t].wait()
        wT = wqkv_v[cols, :].T.astype(f32)
        wts[t][0:1344, :] = wT
        wts[t][1344:1352, :] = jnp.zeros((8, w), f32)
        wp_s[0:448, cols] = wT[0:448].astype(bf)
        wp_s[960:1408, cols] = wT[896:1344].astype(bf)
        for hh in range(H):
            wp_s[448 + 32 * hh:448 + 32 * hh + 32, cols] = wts[t][pl.ds(448 + 28 * hh, 32), :].astype(bf)

    zpad = jnp.zeros((4, 512), f32)
    opad = jnp.where(lax.broadcasted_iota(jnp.int32, (4, 512), 0) == 0, np.float32(1.0), np.float32(0.0))

    def proj_body(b, carry):
        t0 = pl.multiple_of(b * 512, 512)
        x_copy(b).wait()
        xb = xT_v[:, pl.ds(t0, 512)]
        kT = jnp.dot(wp_s[448:960, :], xb, preferred_element_type=f32)
        qq = jnp.dot(wp_s[0:448, :], xb, preferred_element_type=f32) * np.float32(DH ** -0.5 * LOG2E)
        for hh in range(H):
            q_s[hh, :, pl.ds(t0, 512)] = jnp.concatenate([qq[28 * hh:28 * hh + 28, :], zpad], axis=0).astype(bf)
        vv = jnp.dot(wp_s[960:1408, :], xb, preferred_element_type=f32)
        for hh in range(H):
            v_s[hh, :, pl.ds(t0, 512)] = jnp.concatenate([vv[28 * hh:28 * hh + 28, :], opad], axis=0).astype(bf)
        for g in range(4):
            kg = kT[128 * g:128 * g + 128, :].T
            k_s[4 * g, pl.ds(t0, 512), :] = kg.astype(bf)
            for j in range(1, 4):
                k_s[4 * g + j, pl.ds(t0, 512), :] = pltpu.roll(kg, 128 - 32 * j, 1).astype(bf)
        return carry
    lax.fori_loop(0, 4, proj_body, 0)

    for c in cp_par:
        c.wait()
    cp_ldt.wait()
    dt_row = jnp.exp(ldt_v[...].astype(f32).reshape(1, D)).astype(bf).astype(f32)
    dt_s[0:D, :] = jnp.broadcast_to(dt_row, (128, D)).T
    cp_cst.wait()
    cp_u.wait()
    cp_dsk.wait()
    cp_wo.wait()
    wo_f[...] = wo_v[...].astype(f32)
    for hh in range(H):
        wop_s[32 * hh:32 * hh + 32, :] = jnp.concatenate(
            [wo_f[28 * hh:28 * hh + 28, :], jnp.zeros((4, D), f32)], axis=0).astype(bf)

    def bprep(r0, n, fast):
        sl = pl.ds(r0, n)
        dtc = dt_s[sl, :]
        dt2 = jnp.concatenate([dtc, dtc], axis=1)
        zr = dt2 * par_v[0, sl, :].astype(f32)
        zi = dt2 * par_v[1, sl, :].astype(f32)
        dbr = dt2 * par_v[2, sl, :].astype(f32)
        dbi = dt2 * par_v[3, sl, :].astype(f32)
        wr, wi = _cmul(par_v[4, sl, :].astype(f32), par_v[5, sl, :].astype(f32), dbr, dbi)
        pw[2, sl, :] = wr
        pw[3, sl, :] = wi
        mag = jnp.exp(zr)
        sn, cs = _sincos(zi) if fast else (jnp.sin(zi), jnp.cos(zi))
        pw[0, sl, :] = mag * cs
        pw[1, sl, :] = mag * sn

    def kgen_prep(b, st):
        d0 = pl.multiple_of(b * 8, 8)
        gs = gss[st]

        def ld(k):
            return pw[k, pl.ds(d0, 8), :], pw[k + 1, pl.ds(d0, 8), :]

        def tmp_ld(k):
            r = 48 * st + 16 * k
            return pw[4, r:r + 8, :], pw[4, r + 8:r + 16, :]

        def tmp_st(k, v):
            r = 48 * st + 16 * k
            pw[4, r:r + 8, :] = v[0]
            pw[4, r + 8:r + 16, :] = v[1]

        def put_rows(rr, ri, val):
            for t in range(2):
                gs[t, rr:rr + 8, :] = val[0][:, 128 * t:128 * t + 128]
                gs[t, ri:ri + 8, :] = val[1][:, 128 * t:128 * t + 128]

        def get_rows(rr, ri):
            return tuple(jnp.concatenate([gs[t, r:r + 8, :] for t in range(2)], axis=1) for r in (rr, ri))

        def put_e(idx, val):
            put_rows(ER + 12 * idx, EI + 12 * idx, val)

        def put_p(idx, val):
            put_rows(PR + 12 * idx, PI + 12 * idx, val)

        def get_p(idx):
            return get_rows(PR + 12 * idx, PI + 12 * idx)

        e1, w = ld(0), ld(2)
        put_e(0, w)
        put_e(1, _cmul(*w, *e1))
        e2 = _csq(*e1)
        put_e(2, _cmul(*w, *e2))
        tmp_st(0, e2)
        tmp_st(1, _cmul(*e2, *e1))
        yield
        w, e2, e3 = ld(2), tmp_ld(0), tmp_ld(1)
        put_e(3, _cmul(*w, *e3))
        e4 = _csq(*e2)
        tmp_st(2, e4)
        put_e(4, _cmul(*w, *e4))
        put_e(6, _cmul(*w, *_csq(*e3)))
        yield
        e1, w, e3, e4 = ld(0), ld(2), tmp_ld(1), tmp_ld(2)
        put_e(5, _cmul(*w, *_cmul(*e4, *e1)))
        put_e(7, _cmul(*w, *_cmul(*e4, *e3)))
        e8 = _csq(*e4)
        put_p(0, (jnp.ones_like(e8[0]), jnp.zeros_like(e8[0])))
        put_p(1, (e8[0], -e8[1]))
        yield
        p1 = get_p(1)
        p2 = _csq(*p1)
        put_p(2, p2)
        p3 = _cmul(*p2, *p1)
        put_p(3, p3)
        p4 = _csq(*p2)
        put_p(4, p4)
        put_p(5, _cmul(*p4, *p1))
        put_p(6, _csq(*p3))
        yield
        p3, p4 = get_p(3), get_p(4)
        put_p(7, _cmul(*p4, *p3))
        m8 = _csq(*p4)
        put_rows(MU, MU + 8, m8)
        m16 = _csq(*m8)
        put_rows(MU + 16, MU + 24, m16)
        put_rows(MU + 32, MU + 40, _csq(*m16))
        yield
        w, e4, m32 = ld(2), tmp_ld(2), get_rows(MU + 32, MU + 40)
        x512 = _csq(*m32)
        w512 = _cmulc(*w, *x512)
        put_e(8, w512)
        put_e(9, _cmul(*w512, *e4))
        x1024 = _csq(*x512)
        put_e(10, _cmulc(*w, *x1024))
        put_e(11, _cmulc(*w, *_cmul(*x1024, *x512)))
        put_e(12, _cmulc(*w, *_csq(*x1024)))
        yield

    def kgen_chan(b, i, st):
        gs = gss[st]
        e2_r, e2_i, e1_r, e1_i = [], [], [], []
        for t in range(2):
            b0 = (gs[t, pl.ds(PR + i, 8, stride=12), :], gs[t, pl.ds(PI + i, 8, stride=12), :])
            m8, m16, m32 = [(jnp.broadcast_to(gs[t, pl.ds(MU + 16 * k + i, 1), :], (8, 128)),
                             jnp.broadcast_to(gs[t, pl.ds(MU + 16 * k + 8 + i, 1), :], (8, 128)))
                            for k in range(3)]
            b1 = _cmul(*b0, *m8)
            b2 = _cmul(*b0, *m16)
            b3 = _cmul(*b1, *m16)
            blks = (b0, b1, b2, b3, _cmul(*b0, *m32), _cmul(*b1, *m32), _cmul(*b2, *m32), _cmul(*b3, *m32))
            e2_r.append(jnp.concatenate([v[0] for v in blks], axis=0))
            e2_i.append(jnp.concatenate([v[1] for v in blks], axis=0))
            e1_r.append(gs[t, pl.ds(ER + i, 16, stride=12), :])
            e1_i.append(gs[t, pl.ds(EI + i, 16, stride=12), :])
        lhs = jnp.concatenate(e1_r + e1_i, axis=1).astype(bf)
        rhs = jnp.concatenate(e2_r + e2_i, axis=1).astype(bf)
        kc = lax.dot_general(lhs, rhs, _NT, preferred_element_type=f32)
        xk_s[pl.ds(64 + b * 8 + i, 16, stride=XP), :] = kc

    def put_spectrum(which, idx, val):
        for lt in range(4):
            kuh[which, lt, idx, 0:128, :] = val[0:128, 128 * lt:128 * lt + 128]
            kuh[which, lt, idx, IMO:IMO + 128, :] = val[128:256, 128 * lt:128 * lt + 128]

    def u_fwd(a):
        t0 = pl.multiple_of(a * 128, 128)
        put_spectrum(1, a, lax.dot_general(cst_v[0], uT_s[:, pl.ds(t0, 128)], _NT, preferred_element_type=f32))

    def k_tr(rho):
        r0 = pl.multiple_of(rho * XP, 4)
        c0 = pl.multiple_of(rho * 64, 64)
        kct_s[pl.ds(c0, 64), :] = xk_s[pl.ds(r0, 512), :].astype(bf).T

    def k_fwd(j):
        g = jnp.where(j < 2, 1, jnp.where(j < 4, 2, jnp.where(j < 8, 3, 4)))
        win = jnp.concatenate(
            [kct_s[pl.ds(pl.multiple_of(tab_s[j * 8 + si], 16), 16), :] for si in range(8)], axis=0)
        put_spectrum(0, j, jnp.dot(cst_v[g], win, preferred_element_type=f32))

    def conv_pair(unit, p):
        lt = unit // 16
        r0 = pl.multiple_of((unit % 16) * 8, 8)

        def ld(which, idx):
            return kuh[which, lt, idx, pl.ds(r0, 8), :], kuh[which, lt, idx, pl.ds(IMO + r0, 8), :]

        def mac(acc, k, u):
            t = (k[0] * u[0] - k[1] * u[1], k[0] * u[1] + k[1] * u[0])
            return t if acc is None else (acc[0] + t[0], acc[1] + t[1])
        a0, a1 = 2 * p, 2 * p + 1
        y0 = y1 = uprev = None
        cuts = set(int(round((a1 + 1) * k / NPIN_C)) for k in range(1, NPIN_C))
        for j in range(a1 + 1):
            if j in cuts:
                yield
            k = ld(0, j)
            y1 = mac(y1, k, ld(1, a1 - j) if uprev is None else uprev)
            if a0 - j >= 0:
                uprev = ld(1, a0 - j)
                y0 = mac(y0, k, uprev)
        for a, y in ((a0, y0), (a1, y1)):
            yf_s[a + 1, lt, pl.ds(r0, 8), :] = y[0]
            yf_s[a + 1, lt, pl.ds(IMO + r0, 8), :] = y[1]
        yield

    cinv = jnp.concatenate([cst_v[5, 0:128, :], cst_v[5, 128:256, :]], axis=1)
    sgn = jnp.where(lax.broadcasted_iota(jnp.int32, (128, 128), 0) % 2 == 0, np.float32(1.0), np.float32(-1.0))

    def inverse(a):
        t0 = pl.multiple_of(a * 128, 128)
        parts = []
        for lt in range(4):
            yr = yf_s[a + 1, lt, 0:128, :] - sgn * yf_s[a, lt, IMO:IMO + 128, :]
            yi = yf_s[a + 1, lt, IMO:IMO + 128, :] + sgn * yf_s[a, lt, 0:128, :]
            parts.append(jnp.concatenate([yr, yi], axis=0).astype(bf))
        y = jnp.dot(cinv, jnp.concatenate(parts, axis=1), preferred_element_type=f32).astype(bf)
        st_s[pl.ds(t0, 128), 448:512] = y[:, 64:128]
        st_s[pl.ds(t0, 128), 512:896] = y[:, 128:512]

    def ex_P(i, c, state, fast):
        tasks = [_task(u_fwd, i * 4 + c // 4)] if c % 4 == 1 else []
        if not fast:
            if c in (0, 8):
                r0 = pl.multiple_of(i * 112 + (0 if c == 0 else 48), 16)
                tasks.append(_task(bprep, r0, 48 if c == 0 else 64, False))
            return None, tasks
        if c >= 14:
            return None, tasks
        spare = pl.multiple_of(D + _opaque0(i, 9) * 16, 16)

        def pin(v):
            dt_s[pl.ds(spare, 8), :] = v
            par_v[0, pl.ds(spare, 16), 0:128] = jnp.concatenate([v, v], axis=0).astype(bf)
        return (pin, 1, [_task(bprep, pl.multiple_of(i * 112 + 8 * c, 8), 8, True)]), tasks

    def ex_G(i, c, state):
        j = i - I_G
        st = c // 8
        spare = pl.multiple_of(D + _opaque0(i, 9) * 8, 8)

        def pin(v):
            pw[4, pl.ds(spare, 8), 0:128] = v
        tasks = [_task(kgen_chan, 2 * j + st, c % 8, st)]
        if c % 8 == 0:
            state['prep'] = kgen_prep(2 * j + 1 if st == 0 else jnp.minimum(2 * j + 2, D // 8 - 1), 1 - st)
        if c % 8 < 6:
            return (pin, 1, [_task(next, state['prep'])]), tasks
        return None, tasks

    def outproj(r0, n):
        oT = o_s[:, :, pl.ds(r0, n)].reshape(512, n)
        ya = lax.dot_general(oT, wop_s[...], _TN, preferred_element_type=f32)
        st_s[pl.ds(r0, n), 0:448] = ya.astype(bf)

    def ex_T(i, c, state):
        tasks = [_task(k_tr, (i - I_T) * 4 + c // 4)] if c % 4 == 1 else []
        if c == OPC:
            tasks.append(_task(outproj, pl.multiple_of((i - I_T) * 256, 256), 256))
        return None, tasks

    def ex_KF(i, c, state):
        return None, ([_task(k_fwd, (i - I_KF) * 4 + c // 4)] if c % 4 == 1 else [])

    def ex_C(i, c, state):
        spare = 16 + _opaque0(i, 9)

        def pin(v):
            kuh[0, 0, spare, 0:8, :] = v
        unit = (i - I_C) * 4 + c // 4
        return (pin, NPIN_C, [conv_pair(unit, c % 4), conv_pair(unit, 7 - c % 4)]), []

    def ex_I(i, c, state):
        return None, ([_task(inverse, (i - I_I) * 2 + c // 8)] if c % 8 == 2 else [])

    def out_copy(qb):
        q0 = pl.multiple_of(qb * BQ, BQ)
        return pltpu.make_async_copy(st_s.at[pl.ds(q0, BQ), :], out_h.at[0, pl.ds(q0, BQ), :], osem.at[qb])

    def q_of(i):
        return q_s[i % H, :, pl.ds(pl.multiple_of((i // H) * BQ, BQ), BQ)], i % H

    def pv_chunk(h, c, m, acc):
        p = jnp.exp2(s_s[pl.ds(c * CK, CK), :] - m).astype(bf)
        o = jnp.dot(v_s[h, :, pl.ds(c * CK, CK)], p, preferred_element_type=f32)
        return o if acc is None else acc + o

    def qk_chunk(h, q, c):
        return jnp.dot(k_s[h, pl.ds(c * CK, CK), 0:32], q, preferred_element_type=f32)

    def qk_keep(s, c, mrun, pins=None, tasks=()):
        s_s[pl.ds(c * CK, CK), :] = s
        mm = jnp.max(s.reshape(CK // 8, 8, BQ), axis=0)
        if pins is not None:
            pin, npin, pinned = pins
            for k in range(npin):
                g = (k + 1) * (CK // 8) // npin - 1
                pin(s[8 * g:8 * g + 8, 0:128])
                for t in pinned:
                    next(t, None)
            _drain(pinned)
        _drain(tasks)
        return mm if mrun is None else jnp.maximum(mrun, mm)

    def att_step(i, mrun_prev, extra, nqf, last=False):
        m = jnp.max(mrun_prev, axis=0, keepdims=True)
        if not last:
            qn, hn = q_of(jnp.minimum(i + 1, NB - 1))
        h = i % H
        mrun = acc = None
        state = {}
        for c in range(NC):
            if last:
                acc = pv_chunk(h, c, m, acc)
                _drain(extra(i, c, state)[1])
                continue
            if c < nqf:
                s = qk_chunk(hn, qn, c)
                acc = pv_chunk(h, c, m, acc)
            else:
                acc = pv_chunk(h, c, m, acc)
                s = qk_chunk(hn, qn, c)
            mrun = qk_keep(s, c, mrun, *extra(i, c, state))
        inv = 1.0 / acc[28:29, :]
        o_s[h, :, pl.ds(pl.multiple_of((i // H) * BQ, BQ), BQ)] = (acc * inv).astype(bf)
        return mrun

    def run(lo, hi, extra, mrun, nqf, unroll=1, pre=None):
        def body(t, mrun):
            if pre is not None:
                pre(t)
            for u in range(unroll):
                mrun = att_step(t * unroll + u, mrun, extra, nqf)
            return mrun
        return lax.fori_loop(lo // unroll, hi // unroll, body, mrun)

    q0, _ = q_of(0)
    mrun = None
    for c in range(NC):
        mrun = qk_keep(qk_chunk(0, q0, c), c, mrun)

    zmax = jnp.max(jnp.abs(par_v[1, 0:D, :].astype(f32)) * jnp.concatenate([dt_s[0:D, :]] * 2, axis=1))
    mr_s[...] = mrun

    @pl.when(zmax <= np.float32(8192.0))
    def _():
        mr_s[...] = run(0, I_G, functools.partial(ex_P, fast=True), mr_s[...], 0)

    @pl.when(jnp.logical_not(zmax <= np.float32(8192.0)))
    def _():
        mr_s[...] = run(0, I_G, functools.partial(ex_P, fast=False), mr_s[...], 0)

    mrun = mr_s[...]
    _drain([kgen_prep(0, 0)])
    mrun = run(I_G, I_T, ex_G, mrun, 3, unroll=2)
    mrun = run(I_T, I_KF, ex_T, mrun, 2)
    mrun = run(I_KF, I_C, ex_KF, mrun, 2)
    dsk = jnp.concatenate([jnp.zeros((1, 64), f32), dsk_v[...].astype(f32).reshape(1, D)], axis=1)
    for lt in range(4):
        kuh[0, lt, 0, 0:128, :] = kuh[0, lt, 0, 0:128, :] + dsk[:, 128 * lt:128 * lt + 128]
    mrun = run(I_C, I_I, ex_C, mrun, 16, unroll=2)

    def early_store(i):
        @pl.when(jnp.logical_or(i == I_I + 2, i == I_I + 4))
        def _():
            out_copy((i - I_I - 2) // 2).start()
    mrun = run(I_I, NB - 1, ex_I, mrun, 2, pre=early_store)
    att_step(NB - 1, mrun, ex_I, 0, last=True)

    def outproj_body(qb, carry):
        outproj(pl.multiple_of(qb * BQ, BQ), BQ)
        out_copy(qb).start()
        return carry
    lax.fori_loop(2, NQB, outproj_body, 0)
    for qb in range(NQB):
        out_copy(qb).wait()


@jax.jit
def pallas_concat_heads__mha_block__ssm_conv_s4__prompt_kernel(
    A_x: jax.Array,
    A_wqkv: jax.Array,
    A_wo: jax.Array,
    B_u: jax.Array,
    B_A_re: jax.Array,
    B_A_im: jax.Array,
    B_B_re: jax.Array,
    B_B_im: jax.Array,
    B_C_re: jax.Array,
    B_C_im: jax.Array,
    B_log_dt: jax.Array,
    B_Dskip: jax.Array,
):
    scratch = [
        pltpu.VMEM((D, SEQ), bf),
        pltpu.VMEM((D, 3 * D), bf),
        pltpu.VMEM((D, D), bf),
        pltpu.VMEM((512, SEQ), bf),
        pltpu.VMEM((6, D + 16, NST), bf),
        pltpu.VMEM((D,), bf),
        pltpu.VMEM((D,), bf),
        pltpu.VMEM((6, 256, 128), bf),
        pltpu.VMEM((1352, 128), f32),
        pltpu.VMEM((1352, 128), f32),
        pltpu.VMEM((1352, 128), f32),
        pltpu.VMEM((1352, 64), f32),
        pltpu.VMEM((1408, D), bf),
        pltpu.VMEM((D, D), f32),
        pltpu.VMEM((512, D), bf),
        pltpu.VMEM((H, 32, SEQ), bf),
        pltpu.VMEM((H, SEQ, 128), bf),
        pltpu.VMEM((H, 32, SEQ), bf),
        pltpu.VMEM((SEQ, BQ), f32),
        pltpu.VMEM((H, 32, SEQ), bf),
        pltpu.VMEM((5, D + 8, NST), f32),
        pltpu.VMEM((2, 640, 128), f32),
        pltpu.VMEM((2, 640, 128), f32),
        pltpu.VMEM((XP * 16, 64), f32),
        pltpu.VMEM((1024, 512), bf),
        pltpu.VMEM((2, 4, 17, PLN, 128), f32),
        pltpu.VMEM((17, 4, PLN, 128), f32),
        pltpu.VMEM((SEQ, 2 * D), bf),
        pltpu.VMEM((D + 16, 128), f32),
        pltpu.VMEM((8, BQ), f32),
        pltpu.SMEM((128,), jnp.int32),
        pltpu.SemaphoreType.DMA((21,)),
        pltpu.SemaphoreType.DMA((NQB,)),
    ]
    hbm = pl.BlockSpec(memory_space=pltpu.HBM)
    operands = (jnp.transpose(A_x[0]), A_wqkv, A_wo, jnp.transpose(B_u[0]), B_A_re, B_A_im, B_B_re, B_B_im,
                B_C_re, B_C_im, B_log_dt, B_Dskip, jnp.asarray(_CONSTS))
    return pl.pallas_call(
        _kernel,
        out_shape=jax.ShapeDtypeStruct((1, SEQ, 2 * D), bf),
        in_specs=[hbm] * len(operands),
        out_specs=hbm,
        scratch_shapes=scratch,
        compiler_params=pltpu.CompilerParams(vmem_limit_bytes=110 * 2 ** 20),
    )(*[pltpu.with_memory_space_constraint(a, pltpu.HBM) for a in operands])
```

```python
import functools

import jax
import jax.numpy as jnp
import ml_dtypes
import numpy as np
from jax import lax
from jax.experimental import pallas as pl
from jax.experimental.pallas import tpu as pltpu

bf = jnp.bfloat16
f32 = jnp.float32

SEQ = 2048
D = 448
H = 16
DH = 28
NST = 256
BQ = 512
CK = 128
NQB = SEQ // BQ
NB = NQB * H
NC = SEQ // CK
LOG2E = 1.4426950408889634

XP = 516
IMO = 144
PLN = 280
LC0, LC1 = 1, 9
OPC = 7
NPIN_C = 8
PR, PI, ER, EI, MU = 0, 96, 192, 384, 576
I_G, I_T, I_KF, I_C, I_I = 4, 32, 36, 40, 56

_L1 = np.array([0, 1, 2, 3, 4, 5, 6, 7, 512, 516, 1024, 1536, 2048])


def _slabs(j):
    if j < 2:
        return [(r, 16 * j) for r in range(8)]
    if j < 4:
        return [(r, 16 * j) for r in (0, 2, 4, 6)] + [(0, 48) if j == 2 else (8, 0)]
    if j < 8:
        return [(8, 16 * (j - 4)), (9, 16 * (j - 4))] + [(8, 16 * (j - 3)) if j < 7 else (10, 0)]
    if j < 12:
        return [(10, 16 * (j - 8))] + [(10, 16 * (j - 7)) if j < 11 else (11, 0)]
    return [(11, 16 * (j - 12))] + [(11, 16 * (j - 11)) if j < 15 else (12, 0)]


def _slab_rows(j):
    rows = [64 * rho + c0 for rho, c0 in _slabs(j)]
    return rows + [rows[0]] * (8 - len(rows))


def _make_consts():
    k = np.arange(128)[:, None]
    n = np.arange(128)[None, :]
    ang = np.pi * (2 * k + 1) * n / 256.0
    ct = np.concatenate([np.cos(ang), -np.sin(ang)], 0)
    ci = np.concatenate([np.cos(ang.T), -np.sin(ang.T)], 1) / 128.0
    out = np.zeros((6, 256, 128), np.float64)
    out[0] = ct
    for g, j in enumerate((0, 2, 4, 8)):
        pos = {}
        for si, (rho, c0) in enumerate(_slabs(j)):
            for cc in range(16):
                pos.setdefault(int(_L1[rho] + 8 * (c0 + cc)), si * 16 + cc)
        for nn in range(128):
            lag = int(np.float32(128 * j + nn).astype(ml_dtypes.bfloat16).astype(np.float32))
            out[g + 1][:, pos[lag]] += ct[:, nn]
    out[5, 0:128] = ci[:, 0:128]
    out[5, 128:256] = ci[:, 128:256]
    return out.astype(np.float32).astype(ml_dtypes.bfloat16)


_CONSTS = _make_consts()


def _cmul(ar, ai, br, bi):
    return ar * br - ai * bi, ar * bi + ai * br


def _cmulc(ar, ai, br, bi):
    return ar * br + ai * bi, ai * br - ar * bi


def _csq(ar, ai):
    return ar * ar - ai * ai, (ar + ar) * ai


def _sincos(x):
    kf = jnp.round(x * np.float32(2.0 / np.pi))
    ki = kf.astype(jnp.int32)
    r = x - kf * np.float32(1.5703125)
    r = r - kf * np.float32(4.837512969970703125e-4)
    r = r - kf * np.float32(7.54978995489188216e-8)
    r2 = r * r
    s = r + r * r2 * (np.float32(-1.6666654611e-1)
                      + r2 * (np.float32(8.3321608736e-3) + r2 * np.float32(-1.9515295891e-4)))
    c = (np.float32(1.0) - np.float32(0.5) * r2) + r2 * r2 * (
        np.float32(4.166664568298827e-2)
        + r2 * (np.float32(-1.388731625493765e-3) + r2 * np.float32(2.443315711809948e-5)))
    swap = (ki & 1) == 1
    sb = jnp.where(swap, c, s)
    cb = jnp.where(swap, s, c)
    return jnp.where((ki & 2) != 0, -sb, sb), jnp.where(((ki + 1) & 2) != 0, -cb, cb)


def _task(fn, *args):
    def g():
        fn(*args)
        yield
    return g()


def _drain(tasks):
    for t in tasks:
        for _ in t:
            pass


def _opaque0(i, k):
    return (i * k) >> 12


_NT = (((1,), (1,)), ((), ()))
_TN = (((0,), (0,)), ((), ()))


def _kernel(xT_h, wqkv_h, wo_h, uT_h, are_h, aim_h, bre_h, bim_h, cre_h, cim_h, ldt_h, dsk_h, cst_h,
            out_h,
            xT_v, wqkv_v, wo_v, uT_s, par_v, ldt_v, dsk_v, cst_v,
            wt0, wt1, wt2, wt3, wp_s, wo_f, wop_s,
            q_s, k_s, v_s, s_s, o_s,
            pw, gs0, gs1, xk_s, kct_s, kuh, yf_s, st_s, dt_s, mr_s, tab_s, sems, osem):
    gss = (gs0, gs1)
    wts = (wt0, wt1, wt2, wt3)

    def w_copy(c0, n, k):
        return pltpu.make_async_copy(wqkv_h.at[:, pl.ds(c0, n)], wqkv_v.at[:, pl.ds(c0, n)], sems.at[17 + k])
    cp_wk, cp_wq, cp_wv = w_copy(384, 512, 0), w_copy(0, 384, 1), w_copy(896, 448, 2)

    def x_copy(b):
        t0 = pl.multiple_of(b * 512, 512)
        return pltpu.make_async_copy(xT_h.at[:, pl.ds(t0, 512)], xT_v.at[:, pl.ds(t0, 512)], sems.at[13 + b])
    cp_par = [pltpu.make_async_copy(r, par_v.at[i, pl.ds(0, D), :], sems.at[2 + i])
              for i, r in enumerate((are_h, aim_h, bre_h, bim_h, cre_h, cim_h))]
    cp_ldt = pltpu.make_async_copy(ldt_h, ldt_v, sems.at[8])
    cp_dsk = pltpu.make_async_copy(dsk_h, dsk_v, sems.at[9])
    cp_cst = pltpu.make_async_copy(cst_h, cst_v, sems.at[10])
    cp_wo = pltpu.make_async_copy(wo_h, wo_v, sems.at[11])
    cp_u = pltpu.make_async_copy(uT_h, uT_s.at[pl.ds(64, D), :], sems.at[12])
    cp_wk.start()
    x_copy(0).start()
    cp_wq.start()
    cp_wv.start()
    x_copy(1).start()
    for c in cp_par:
        c.start()
    cp_ldt.start()
    x_copy(2).start()
    x_copy(3).start()
    cp_dsk.start()
    cp_cst.start()
    cp_wo.start()
    cp_u.start()

    uT_s[0:64, :] = jnp.zeros((64, SEQ), bf)
    for j in range(16):
        for si, r in enumerate(_slab_rows(j)):
            tab_s[j * 8 + si] = np.int32(r)
    for gs in gss:
        for t in range(2):
            gs[t, ER + 13 * 12:ER + 16 * 12, :] = jnp.zeros((36, 128), f32)
            gs[t, EI + 13 * 12:EI + 16 * 12, :] = jnp.zeros((36, 128), f32)
    for rho in range(16):
        xk_s[XP * rho:XP * rho + 64, :] = jnp.zeros((64, 64), f32)
    for lt in range(4):
        yf_s[0, lt, 0:128, :] = jnp.zeros((128, 128), f32)
        yf_s[0, lt, IMO:IMO + 128, :] = jnp.zeros((128, 128), f32)

    def w_rows(c0, n):
        return wqkv_v[:, c0:c0 + n].T.astype(f32)

    def prep_wk():
        cp_wk.wait()
        for c0 in range(384, 896, 128):
            wT = w_rows(c0, 128)
            if c0 == 384:
                wp_s[384:448, :] = wT[0:64].astype(bf)
                wT = wT[64:128]
            r0 = max(c0 - 448, 0)
            for t in range(4):
                wts[t][r0:r0 + wT.shape[0], :] = wT[:, 128 * t:min(128 * t + 128, D)]
        for t in range(4):
            wts[t][448:456, :] = jnp.zeros((8, 64 if t == 3 else 128), f32)
        for hh in range(H):
            wp_s[448 + 32 * hh:448 + 32 * hh + 32, :] = jnp.concatenate(
                [wts[t][pl.ds(28 * hh, 32), :] for t in range(4)], axis=1).astype(bf)

    def prep_wq():
        cp_wq.wait()
        for c0 in range(0, 384, 128):
            wp_s[c0:c0 + 128, :] = w_rows(c0, 128).astype(bf)

    def prep_wv():
        cp_wv.wait()
        for c0 in range(896, 1344, 128):
            n = min(128, 1344 - c0)
            wp_s[64 + c0:64 + c0 + n, :] = w_rows(c0, n).astype(bf)

    zpad = jnp.zeros((4, 512), f32)
    opad = jnp.where(lax.broadcasted_iota(jnp.int32, (4, 512), 0) == 0, np.float32(1.0), np.float32(0.0))

    def proj_body(b, carry, first=False):
        t0 = b * 512 if first else pl.multiple_of(b * 512, 512)
        x_copy(b).wait()
        xb = xT_v[:, pl.ds(t0, 512)]
        kT = jnp.dot(wp_s[448:960, :], xb, preferred_element_type=f32)
        if first:
            prep_wq()
        qq = jnp.dot(wp_s[0:448, :], xb, preferred_element_type=f32) * np.float32(DH ** -0.5 * LOG2E)
        for hh in range(H):
            q_s[hh, :, pl.ds(t0, 512)] = jnp.concatenate([qq[28 * hh:28 * hh + 28, :], zpad], axis=0).astype(bf)
        if first:
            prep_wv()
        vv = jnp.dot(wp_s[960:1408, :], xb, preferred_element_type=f32)
        for hh in range(H):
            v_s[hh, :, pl.ds(t0, 512)] = jnp.concatenate([vv[28 * hh:28 * hh + 28, :], opad], axis=0).astype(bf)
        for g in range(4):
            kg = kT[128 * g:128 * g + 128, :].T
            k_s[4 * g, pl.ds(t0, 512), :] = kg.astype(bf)
            for j in range(1, 4):
                k_s[4 * g + j, pl.ds(t0, 512), :] = pltpu.roll(kg, 128 - 32 * j, 1).astype(bf)
        return carry
    prep_wk()
    proj_body(0, 0, first=True)
    lax.fori_loop(1, 4, proj_body, 0)

    for c in cp_par:
        c.wait()
    cp_ldt.wait()
    dt_row = jnp.exp(ldt_v[...].astype(f32).reshape(1, D)).astype(bf).astype(f32)
    dt_s[0:D, :] = jnp.broadcast_to(dt_row, (128, D)).T
    cp_cst.wait()
    cp_u.wait()
    cp_dsk.wait()
    cp_wo.wait()
    wo_f[...] = wo_v[...].astype(f32)
    for hh in range(H):
        wop_s[32 * hh:32 * hh + 32, :] = jnp.concatenate(
            [wo_f[28 * hh:28 * hh + 28, :], jnp.zeros((4, D), f32)], axis=0).astype(bf)

    def bprep(r0, n, fast):
        sl = pl.ds(r0, n)
        dtc = dt_s[sl, :]
        dt2 = jnp.concatenate([dtc, dtc], axis=1)
        zr = dt2 * par_v[0, sl, :].astype(f32)
        zi = dt2 * par_v[1, sl, :].astype(f32)
        dbr = dt2 * par_v[2, sl, :].astype(f32)
        dbi = dt2 * par_v[3, sl, :].astype(f32)
        wr, wi = _cmul(par_v[4, sl, :].astype(f32), par_v[5, sl, :].astype(f32), dbr, dbi)
        pw[2, sl, :] = wr
        pw[3, sl, :] = wi
        mag = jnp.exp(zr)
        sn, cs = _sincos(zi) if fast else (jnp.sin(zi), jnp.cos(zi))
        pw[0, sl, :] = mag * cs
        pw[1, sl, :] = mag * sn

    def kgen_prep(b, st):
        d0 = pl.multiple_of(b * 8, 8)
        gs = gss[st]

        def ld(k):
            return pw[k, pl.ds(d0, 8), :], pw[k + 1, pl.ds(d0, 8), :]

        def tmp_ld(k):
            r = 48 * st + 16 * k
            return pw[4, r:r + 8, :], pw[4, r + 8:r + 16, :]

        def tmp_st(k, v):
            r = 48 * st + 16 * k
            pw[4, r:r + 8, :] = v[0]
            pw[4, r + 8:r + 16, :] = v[1]

        def put_rows(rr, ri, val):
            for t in range(2):
                gs[t, rr:rr + 8, :] = val[0][:, 128 * t:128 * t + 128]
                gs[t, ri:ri + 8, :] = val[1][:, 128 * t:128 * t + 128]

        def get_rows(rr, ri):
            return tuple(jnp.concatenate([gs[t, r:r + 8, :] for t in range(2)], axis=1) for r in (rr, ri))

        def put_e(idx, val):
            put_rows(ER + 12 * idx, EI + 12 * idx, val)

        def put_p(idx, val):
            put_rows(PR + 12 * idx, PI + 12 * idx, val)

        def get_p(idx):
            return get_rows(PR + 12 * idx, PI + 12 * idx)

        e1, w = ld(0), ld(2)
        put_e(0, w)
        put_e(1, _cmul(*w, *e1))
        e2 = _csq(*e1)
        put_e(2, _cmul(*w, *e2))
        tmp_st(0, e2)
        tmp_st(1, _cmul(*e2, *e1))
        yield
        w, e2, e3 = ld(2), tmp_ld(0), tmp_ld(1)
        put_e(3, _cmul(*w, *e3))
        e4 = _csq(*e2)
        tmp_st(2, e4)
        put_e(4, _cmul(*w, *e4))
        put_e(6, _cmul(*w, *_csq(*e3)))
        yield
        e1, w, e3, e4 = ld(0), ld(2), tmp_ld(1), tmp_ld(2)
        put_e(5, _cmul(*w, *_cmul(*e4, *e1)))
        put_e(7, _cmul(*w, *_cmul(*e4, *e3)))
        e8 = _csq(*e4)
        put_p(0, (jnp.ones_like(e8[0]), jnp.zeros_like(e8[0])))
        put_p(1, (e8[0], -e8[1]))
        yield
        p1 = get_p(1)
        p2 = _csq(*p1)
        put_p(2, p2)
        p3 = _cmul(*p2, *p1)
        put_p(3, p3)
        p4 = _csq(*p2)
        put_p(4, p4)
        put_p(5, _cmul(*p4, *p1))
        put_p(6, _csq(*p3))
        yield
        p3, p4 = get_p(3), get_p(4)
        put_p(7, _cmul(*p4, *p3))
        m8 = _csq(*p4)
        put_rows(MU, MU + 8, m8)
        m16 = _csq(*m8)
        put_rows(MU + 16, MU + 24, m16)
        put_rows(MU + 32, MU + 40, _csq(*m16))
        yield
        w, e4, m32 = ld(2), tmp_ld(2), get_rows(MU + 32, MU + 40)
        x512 = _csq(*m32)
        w512 = _cmulc(*w, *x512)
        put_e(8, w512)
        put_e(9, _cmul(*w512, *e4))
        x1024 = _csq(*x512)
        put_e(10, _cmulc(*w, *x1024))
        put_e(11, _cmulc(*w, *_cmul(*x1024, *x512)))
        put_e(12, _cmulc(*w, *_csq(*x1024)))
        yield

    def kgen_chan(b, i, st):
        gs = gss[st]
        e2_r, e2_i, e1_r, e1_i = [], [], [], []
        for t in range(2):
            b0 = (gs[t, pl.ds(PR + i, 8, stride=12), :], gs[t, pl.ds(PI + i, 8, stride=12), :])
            m8, m16, m32 = [(jnp.broadcast_to(gs[t, pl.ds(MU + 16 * k + i, 1), :], (8, 128)),
                             jnp.broadcast_to(gs[t, pl.ds(MU + 16 * k + 8 + i, 1), :], (8, 128)))
                            for k in range(3)]
            b1 = _cmul(*b0, *m8)
            b2 = _cmul(*b0, *m16)
            b3 = _cmul(*b1, *m16)
            blks = (b0, b1, b2, b3, _cmul(*b0, *m32), _cmul(*b1, *m32), _cmul(*b2, *m32), _cmul(*b3, *m32))
            e2_r.append(jnp.concatenate([v[0] for v in blks], axis=0))
            e2_i.append(jnp.concatenate([v[1] for v in blks], axis=0))
            e1_r.append(gs[t, pl.ds(ER + i, 16, stride=12), :])
            e1_i.append(gs[t, pl.ds(EI + i, 16, stride=12), :])
        lhs = jnp.concatenate(e1_r + e1_i, axis=1).astype(bf)
        rhs = jnp.concatenate(e2_r + e2_i, axis=1).astype(bf)
        kc = lax.dot_general(lhs, rhs, _NT, preferred_element_type=f32)
        xk_s[pl.ds(64 + b * 8 + i, 16, stride=XP), :] = kc

    def put_spectrum(which, idx, val):
        for lt in range(4):
            kuh[which, lt, idx, 0:128, :] = val[0:128, 128 * lt:128 * lt + 128]
            kuh[which, lt, idx, IMO:IMO + 128, :] = val[128:256, 128 * lt:128 * lt + 128]

    def u_fwd(a):
        t0 = pl.multiple_of(a * 128, 128)
        put_spectrum(1, a, lax.dot_general(cst_v[0], uT_s[:, pl.ds(t0, 128)], _NT, preferred_element_type=f32))

    def k_tr(rho):
        r0 = pl.multiple_of(rho * XP, 4)
        c0 = pl.multiple_of(rho * 64, 64)
        kct_s[pl.ds(c0, 64), :] = xk_s[pl.ds(r0, 512), :].astype(bf).T

    def k_fwd(j):
        g = jnp.where(j < 2, 1, jnp.where(j < 4, 2, jnp.where(j < 8, 3, 4)))
        win = jnp.concatenate(
            [kct_s[pl.ds(pl.multiple_of(tab_s[j * 8 + si], 16), 16), :] for si in range(8)], axis=0)
        put_spectrum(0, j, jnp.dot(cst_v[g], win, preferred_element_type=f32))

    def conv_pair(unit, p):
        lt = unit // 16
        r0 = pl.multiple_of((unit % 16) * 8, 8)

        def ld(which, idx):
            return kuh[which, lt, idx, pl.ds(r0, 8), :], kuh[which, lt, idx, pl.ds(IMO + r0, 8), :]

        def mac(acc, k, u):
            t = (k[0] * u[0] - k[1] * u[1], k[0] * u[1] + k[1] * u[0])
            return t if acc is None else (acc[0] + t[0], acc[1] + t[1])
        a0, a1 = 2 * p, 2 * p + 1
        y0 = y1 = uprev = None
        cuts = set(int(round((a1 + 1) * k / NPIN_C)) for k in range(1, NPIN_C))
        for j in range(a1 + 1):
            if j in cuts:
                yield
            k = ld(0, j)
            y1 = mac(y1, k, ld(1, a1 - j) if uprev is None else uprev)
            if a0 - j >= 0:
                uprev = ld(1, a0 - j)
                y0 = mac(y0, k, uprev)
        for a, y in ((a0, y0), (a1, y1)):
            yf_s[a + 1, lt, pl.ds(r0, 8), :] = y[0]
            yf_s[a + 1, lt, pl.ds(IMO + r0, 8), :] = y[1]
        yield

    cinv = jnp.concatenate([cst_v[5, 0:128, :], cst_v[5, 128:256, :]], axis=1)
    sgn = jnp.where(lax.broadcasted_iota(jnp.int32, (128, 128), 0) % 2 == 0, np.float32(1.0), np.float32(-1.0))

    def inverse(a):
        t0 = pl.multiple_of(a * 128, 128)
        parts = []
        for lt in range(4):
            yr = yf_s[a + 1, lt, 0:128, :] - sgn * yf_s[a, lt, IMO:IMO + 128, :]
            yi = yf_s[a + 1, lt, IMO:IMO + 128, :] + sgn * yf_s[a, lt, 0:128, :]
            parts.append(jnp.concatenate([yr, yi], axis=0).astype(bf))
        y = jnp.dot(cinv, jnp.concatenate(parts, axis=1), preferred_element_type=f32).astype(bf)
        st_s[pl.ds(t0, 128), 448:512] = y[:, 64:128]
        st_s[pl.ds(t0, 128), 512:896] = y[:, 128:512]

    def ex_P(i, c, state, fast):
        tasks = [_task(u_fwd, i * 4 + c // 4)] if c % 4 == 1 else []
        if not fast:
            if c in (0, 8):
                r0 = pl.multiple_of(i * 112 + (0 if c == 0 else 48), 16)
                tasks.append(_task(bprep, r0, 48 if c == 0 else 64, False))
            return None, tasks
        if c >= 14:
            return None, tasks
        spare = pl.multiple_of(D + _opaque0(i, 9) * 16, 16)

        def pin(v):
            dt_s[pl.ds(spare, 8), :] = v
            par_v[0, pl.ds(spare, 16), 0:128] = jnp.concatenate([v, v], axis=0).astype(bf)
        return (pin, 1, [_task(bprep, pl.multiple_of(i * 112 + 8 * c, 8), 8, True)]), tasks

    def ex_G(i, c, state):
        j = i - I_G
        st = c // 8
        spare = pl.multiple_of(D + _opaque0(i, 9) * 8, 8)

        def pin(v):
            pw[4, pl.ds(spare, 8), 0:128] = v
        tasks = [_task(kgen_chan, 2 * j + st, c % 8, st)]
        if c % 8 == 0:
            state['prep'] = kgen_prep(2 * j + 1 if st == 0 else jnp.minimum(2 * j + 2, D // 8 - 1), 1 - st)
        if c % 8 < 6:
            return (pin, 1, [_task(next, state['prep'])]), tasks
        return None, tasks

    def outproj(r0, n):
        oT = o_s[:, :, pl.ds(r0, n)].reshape(512, n)
        ya = lax.dot_general(oT, wop_s[...], _TN, preferred_element_type=f32)
        st_s[pl.ds(r0, n), 0:448] = ya.astype(bf)

    def ex_T(i, c, state):
        tasks = [_task(k_tr, (i - I_T) * 4 + c // 4)] if c % 4 == 1 else []
        if c == OPC:
            tasks.append(_task(outproj, pl.multiple_of((i - I_T) * 256, 256), 256))
        return None, tasks

    def ex_KF(i, c, state):
        return None, ([_task(k_fwd, (i - I_KF) * 4 + c // 4)] if c % 4 == 1 else [])

    def ex_C(i, c, state):
        spare = 16 + _opaque0(i, 9)

        def pin(v):
            kuh[0, 0, spare, 0:8, :] = v
        unit = (i - I_C) * 4 + c // 4
        return (pin, NPIN_C, [conv_pair(unit, c % 4), conv_pair(unit, 7 - c % 4)]), []

    def ex_I(i, c, state):
        return None, ([_task(inverse, (i - I_I) * 2 + c // 8)] if c % 8 == 2 else [])

    def out_copy(qb):
        q0 = pl.multiple_of(qb * BQ, BQ)
        return pltpu.make_async_copy(st_s.at[pl.ds(q0, BQ), :], out_h.at[0, pl.ds(q0, BQ), :], osem.at[qb])

    def q_of(i):
        return q_s[i % H, :, pl.ds(pl.multiple_of((i // H) * BQ, BQ), BQ)], i % H

    def pv_chunk(h, c, m, acc):
        p = jnp.exp2(s_s[pl.ds(c * CK, CK), :] - m).astype(bf)
        o = jnp.dot(v_s[h, :, pl.ds(c * CK, CK)], p, preferred_element_type=f32)
        return o if acc is None else acc + o

    def qk_chunk(h, q, c):
        return jnp.dot(k_s[h, pl.ds(c * CK, CK), 0:32], q, preferred_element_type=f32)

    def qk_keep(s, c, mrun, pins=None, tasks=()):
        s_s[pl.ds(c * CK, CK), :] = s
        mm = jnp.max(s.reshape(CK // 8, 8, BQ), axis=0)
        if pins is not None:
            pin, npin, pinned = pins
            for k in range(npin):
                g = (k + 1) * (CK // 8) // npin - 1
                pin(s[8 * g:8 * g + 8, 0:128])
                for t in pinned:
                    next(t, None)
            _drain(pinned)
        _drain(tasks)
        return mm if mrun is None else jnp.maximum(mrun, mm)

    def att_step(i, mrun_prev, extra, nqf, last=False):
        m = jnp.max(mrun_prev, axis=0, keepdims=True)
        if not last:
            qn, hn = q_of(jnp.minimum(i + 1, NB - 1))
        h = i % H
        mrun = acc = None
        state = {}
        for c in range(NC):
            if last:
                acc = pv_chunk(h, c, m, acc)
                _drain(extra(i, c, state)[1])
                continue
            if c < nqf:
                s = qk_chunk(hn, qn, c)
                acc = pv_chunk(h, c, m, acc)
            else:
                acc = pv_chunk(h, c, m, acc)
                s = qk_chunk(hn, qn, c)
            mrun = qk_keep(s, c, mrun, *extra(i, c, state))
        inv = 1.0 / acc[28:29, :]
        o_s[h, :, pl.ds(pl.multiple_of((i // H) * BQ, BQ), BQ)] = (acc * inv).astype(bf)
        return mrun

    def run(lo, hi, extra, mrun, nqf, unroll=1, pre=None):
        def body(t, mrun):
            if pre is not None:
                pre(t)
            for u in range(unroll):
                mrun = att_step(t * unroll + u, mrun, extra, nqf)
            return mrun
        return lax.fori_loop(lo // unroll, hi // unroll, body, mrun)

    q0, _ = q_of(0)
    mrun = None
    for c in range(NC):
        mrun = qk_keep(qk_chunk(0, q0, c), c, mrun)

    zmax = jnp.max(jnp.abs(par_v[1, 0:D, :].astype(f32)) * jnp.concatenate([dt_s[0:D, :]] * 2, axis=1))
    mr_s[...] = mrun

    @pl.when(zmax <= np.float32(8192.0))
    def _():
        mr_s[...] = run(0, I_G, functools.partial(ex_P, fast=True), mr_s[...], 0)

    @pl.when(jnp.logical_not(zmax <= np.float32(8192.0)))
    def _():
        mr_s[...] = run(0, I_G, functools.partial(ex_P, fast=False), mr_s[...], 0)

    mrun = mr_s[...]
    _drain([kgen_prep(0, 0)])
    mrun = run(I_G, I_T, ex_G, mrun, 3, unroll=2)
    mrun = run(I_T, I_KF, ex_T, mrun, 2)
    mrun = run(I_KF, I_C, ex_KF, mrun, 2)
    dsk = jnp.concatenate([jnp.zeros((1, 64), f32), dsk_v[...].astype(f32).reshape(1, D)], axis=1)
    for lt in range(4):
        kuh[0, lt, 0, 0:128, :] = kuh[0, lt, 0, 0:128, :] + dsk[:, 128 * lt:128 * lt + 128]
    mrun = run(I_C, I_I, ex_C, mrun, 16, unroll=2)

    def early_store(i):
        @pl.when(jnp.logical_or(i == I_I + 2, i == I_I + 4))
        def _():
            out_copy((i - I_I - 2) // 2).start()
    mrun = run(I_I, NB - 1, ex_I, mrun, 2, pre=early_store)

    def ex_last(i, c, state):
        tasks = ex_I(i, c, state)[1]
        if c in (LC0, LC1):
            tasks.append(_task(outproj, 2 * BQ + (256 if c == LC1 else 0), 256))
        return None, tasks
    att_step(NB - 1, mrun, ex_last, 0, last=True)

    out_copy(2).start()
    outproj(3 * BQ, BQ)
    out_copy(3).start()
    for qb in range(NQB):
        out_copy(qb).wait()


@jax.jit
def pallas_concat_heads__mha_block__ssm_conv_s4__prompt_kernel(
    A_x: jax.Array,
    A_wqkv: jax.Array,
    A_wo: jax.Array,
    B_u: jax.Array,
    B_A_re: jax.Array,
    B_A_im: jax.Array,
    B_B_re: jax.Array,
    B_B_im: jax.Array,
    B_C_re: jax.Array,
    B_C_im: jax.Array,
    B_log_dt: jax.Array,
    B_Dskip: jax.Array,
):
    scratch = [
        pltpu.VMEM((D, SEQ), bf),
        pltpu.VMEM((D, 3 * D), bf),
        pltpu.VMEM((D, D), bf),
        pltpu.VMEM((512, SEQ), bf),
        pltpu.VMEM((6, D + 16, NST), bf),
        pltpu.VMEM((D,), bf),
        pltpu.VMEM((D,), bf),
        pltpu.VMEM((6, 256, 128), bf),
        pltpu.VMEM((456, 128), f32),
        pltpu.VMEM((456, 128), f32),
        pltpu.VMEM((456, 128), f32),
        pltpu.VMEM((456, 64), f32),
        pltpu.VMEM((1408, D), bf),
        pltpu.VMEM((D, D), f32),
        pltpu.VMEM((512, D), bf),
        pltpu.VMEM((H, 32, SEQ), bf),
        pltpu.VMEM((H, SEQ, 128), bf),
        pltpu.VMEM((H, 32, SEQ), bf),
        pltpu.VMEM((SEQ, BQ), f32),
        pltpu.VMEM((H, 32, SEQ), bf),
        pltpu.VMEM((5, D + 8, NST), f32),
        pltpu.VMEM((2, 640, 128), f32),
        pltpu.VMEM((2, 640, 128), f32),
        pltpu.VMEM((XP * 16, 64), f32),
        pltpu.VMEM((1024, 512), bf),
        pltpu.VMEM((2, 4, 17, PLN, 128), f32),
        pltpu.VMEM((17, 4, PLN, 128), f32),
        pltpu.VMEM((SEQ, 2 * D), bf),
        pltpu.VMEM((D + 16, 128), f32),
        pltpu.VMEM((8, BQ), f32),
        pltpu.SMEM((128,), jnp.int32),
        pltpu.SemaphoreType.DMA((21,)),
        pltpu.SemaphoreType.DMA((NQB,)),
    ]
    hbm = pl.BlockSpec(memory_space=pltpu.HBM)
    operands = (jnp.transpose(A_x[0]), A_wqkv, A_wo, jnp.transpose(B_u[0]), B_A_re, B_A_im, B_B_re, B_B_im,
                B_C_re, B_C_im, B_log_dt, B_Dskip, jnp.asarray(_CONSTS))
    return pl.pallas_call(
        _kernel,
        out_shape=jax.ShapeDtypeStruct((1, SEQ, 2 * D), bf),
        in_specs=[hbm] * len(operands),
        out_specs=hbm,
        scratch_shapes=scratch,
        compiler_params=pltpu.CompilerParams(vmem_limit_bytes=110 * 2 ** 20, disable_bounds_checks=True, disable_semaphore_checks=True),
    )(*[pltpu.with_memory_space_constraint(a, pltpu.HBM) for a in operands])
```
